```python
import jax
import jax.numpy as jnp

def _softmax(x, axis=-1):
    return jax.nn.softmax(x, axis=axis)

def _gelu(x):
    return jax.nn.gelu(x, approximate=True)

def _silu(x):
    return jax.nn.silu(x)

def _sigmoid(x):
    return jax.nn.sigmoid(x)

def _layernorm(x, axis=-1, eps=1e-05):
    m = jnp.mean(x, axis=axis, keepdims=True)
    v = jnp.var(x, axis=axis, keepdims=True)
    return (x - m) / jnp.sqrt(v + eps)

def _scatter_add(tgt, idx, src, axis=0):
    return tgt.at[idx].add(src)

def _segment_sum(src, seg, n):
    return jax.ops.segment_sum(src, seg, n)

class _Rng:

    def __init__(self, key):
        self._k = key

    def _next(self):
        self._k, sub = jax.random.split(self._k)
        return sub

    def normal(self, shape):
        return jax.random.normal(self._next(), shape, dtype=jnp.bfloat16)

    def randint(self, lo, hi, shape):
        return jax.random.randint(self._next(), shape, lo, hi, dtype=jnp.int32)

    def uniform(self, shape, lo=0.0, hi=1.0):
        return jax.random.uniform(self._next(), shape, jnp.bfloat16, lo, hi)

    def permutation(self, n):
        return jax.random.permutation(self._next(), n)
kernel_name = 'gated_mix__memory_aug_recurrent_mem_tr__ssm_conv_h3__prompt'

def setup_inputs():
    _rng = _Rng(jax.random.key(int.from_bytes(__import__("os").urandom(4), "little")))
    _w = lambda a: (lambda t: t.astype(jnp.bfloat16) if jnp.issubdtype(t.dtype, jnp.floating) else t)(jnp.asarray(a))

    def _A_setup():
        B, S, Dm = (1, 2048, 640)
        H, Dh = (32, 192)
        M, seg = (8, 32)
        seg = min(seg, S)
        S = S // seg * seg
        return {'x': _w((lambda *s: _rng.normal(s) * 0.05)(B, S, Dm)), 'mem0': _w((lambda *s: _rng.normal(s) * 0.05)(B, M, Dm)), 'Wq': _w((lambda *s: _rng.normal(s) * 0.05)(Dm, H, Dh) * Dm ** (-0.5)), 'Wk': _w((lambda *s: _rng.normal(s) * 0.05)(Dm, H, Dh) * Dm ** (-0.5)), 'Wv': _w((lambda *s: _rng.normal(s) * 0.05)(Dm, H, Dh) * Dm ** (-0.5)), 'Wo': _w((lambda *s: _rng.normal(s) * 0.05)(H, Dh, Dm) * (H * Dh) ** (-0.5)), 'seg_len': seg}
    _A_in = _A_setup()

    def _B_setup():
        B, S, D = (1, 2048, 640)
        ks = 4
        return {'q': _w((lambda *s: _rng.normal(s) * 0.05)(B, S, D)), 'k': _w((lambda *s: _rng.normal(s) * 0.05)(B, S, D)), 'v': _w((lambda *s: _rng.normal(s) * 0.05)(B, S, D)), 'shift_k': _w((lambda *s: _rng.normal(s) * 0.05)(D, ks) * 0.5), 'ssm_k': _w((lambda *s: _rng.normal(s) * 0.05)(D, S) * (1.0 / S ** 0.5)), 'ssm_D': _w((lambda *s: _rng.normal(s) * 0.05)(D))}
    _B_in = _B_setup()
    return {'A_x': _A_in['x'], 'A_mem0': _A_in['mem0'], 'A_Wq': _A_in['Wq'], 'A_Wk': _A_in['Wk'], 'A_Wv': _A_in['Wv'], 'A_Wo': _A_in['Wo'], 'A_seg_len': _A_in['seg_len'], 'B_q': _B_in['q'], 'B_k': _B_in['k'], 'B_v': _B_in['v'], 'B_shift_k': _B_in['shift_k'], 'B_ssm_k': _B_in['ssm_k'], 'B_ssm_D': _B_in['ssm_D'], 'gate_w': _w((lambda *s: _rng.normal(s) * 0.05)(640))}

def reference(A_x, A_mem0, A_Wq, A_Wk, A_Wv, A_Wo, A_seg_len, B_q, B_k, B_v, B_shift_k, B_ssm_k, B_ssm_D, gate_w):

    def _A_ref(x, mem0, Wq, Wk, Wv, Wo, seg_len):
        B, S, Dm = x.shape
        H, Dh = (Wq.shape[1], Wq.shape[2])
        M = mem0.shape[1]
        scale = Dh ** (-0.5)
        n_seg = S // seg_len
        L = M + seg_len
        idx = jnp.arange(L)
        mask = (idx[:, None] < M) | (idx[:, None] >= idx[None, :])
        mem = mem0
        outs = []
        for s in range(n_seg):
            xs = x[:, s * seg_len:(s + 1) * seg_len, :].copy()
            h = jnp.concatenate([mem, xs], axis=1)
            q = jnp.einsum('btd,dhe->bhte', h, Wq)
            k = jnp.einsum('btd,dhe->bhte', h, Wk)
            v = jnp.einsum('btd,dhe->bhte', h, Wv)
            scores = jnp.einsum('bhqe,bhke->bhqk', q, k) * scale
            scores = jnp.where(mask[None, None], scores, -1000000000.0)
            p = _softmax(scores, axis=-1)
            o = jnp.einsum('bhqk,bhke->bhqe', p, v)
            o = jnp.einsum('bhte,hed->btd', o, Wo)
            mem = o[:, :M, :].copy()
            outs.append(o[:, M:, :])
        return jnp.concatenate(outs, axis=1)

    def _B_ref(q, k, v, shift_k, ssm_k, ssm_D):
        B, S, D = q.shape
        ks = shift_k.shape[-1]
        k_pad = jnp.pad(k, ((0, 0), (ks - 1, 0), (0, 0)))
        k_shift = jnp.zeros_like(k)
        for t in range(ks):
            k_shift = k_shift + k_pad[:, t:t + S, :] * shift_k[:, ks - 1 - t][None, None, :]
        kv = k_shift * v
        L = 2 * S
        kv_pad = jnp.pad(kv, ((0, 0), (0, S), (0, 0)))
        kf_pad = jnp.pad(ssm_k, ((0, 0), (0, S)))
        kv_f = (lambda x, axes=(-2, -1): jnp.fft.rfft2(x.astype(jnp.float32), axes=axes))(kv_pad[:, None, :, :], axes=(1, 2))
        kf_f = (lambda x, axes=(-2, -1): jnp.fft.rfft2(x.astype(jnp.float32), axes=axes))(kf_pad[:, None, :], axes=(1, 2))
        kf_f = (lambda x, *d: x.transpose(*d))(kf_f, 1, 2, 0)
        y_f = kv_f * kf_f[None, :, :, :]
        y = (lambda x, s, axes=(-2, -1): jnp.fft.irfft2(x, s=s, axes=axes).astype(jnp.bfloat16))(y_f, (1, L), axes=(1, 2))[:, 0, :S, :]
        y = y + kv * ssm_D[None, None, :]
        return q * y
    x = A_x
    g = _sigmoid((x * gate_w).sum(-1, keepdims=True))
    a = _A_ref(x, A_mem0, A_Wq, A_Wk, A_Wv, A_Wo, A_seg_len)
    b = _B_ref(x, B_k, B_v, B_shift_k, B_ssm_k, B_ssm_D)
    return g * a + (1 - g) * b
```

```python
import functools

import jax
import jax.experimental.pallas as pl
import jax.experimental.pallas.tpu as pltpu
import jax.numpy as jnp
import numpy as np
from jax import lax

F32 = jnp.float32
BF16 = jnp.bfloat16
I32 = jnp.int32
LANES = 128
CHUNK = 128


def _dft_matrices(c):
    theta = np.pi * (np.arange(c)[:, None] + 0.5) * np.arange(c)[None, :] / c
    fwd = np.concatenate([np.cos(theta), -np.sin(theta)], axis=0)
    inv = np.concatenate([np.cos(theta).T, -np.sin(theta).T], axis=1) / c
    return fwd.astype(np.float32), inv.astype(np.float32)


_FWD, _INV = _dft_matrices(CHUNK)
_NT = (((1,), (1,)), ((), ()))


def _kernel(
    mem0_ref, shift_ref, ssmd_ref, gate_ref, fwd_ref, inv_ref,
    x_hbm, k_hbm, v_hbm, ssm_hbm, wq_hbm, wk_hbm, wv_hbm, wo_hbm,
    out_hbm,
    x_s, k_s, v_s, ssm_s, stage_s, wqkv_s, wo_s,
    kpad_s, kv_s, xf_s, kf_s, zf_s, b_s,
    h_s, q_s, kb_s, vb_s, p_s, o_s, out_s,
    in_sems, w_sems, out_sem,
    *, seq, dm, heads, dh, nmem, seg,
):
    feat = heads * dh
    rows = nmem + seg
    nseg = seq // seg
    pairs = heads // 2
    pw = 2 * dh
    nchunk = seq // CHUNK
    nblk = dm // LANES
    half = CHUNK
    wparts = 4
    wrows = feat // wparts
    w_hbm = (wq_hbm, wk_hbm, wv_hbm, wo_hbm)

    in_copies = [
        pltpu.make_async_copy(src, dst, in_sems.at[i])
        for i, (src, dst) in enumerate(
            ((ssm_hbm, ssm_s), (k_hbm, k_s), (v_hbm, v_s), (x_hbm, x_s))
        )
    ]

    def w_copy(m, part):
        sl = pl.ds(part * wrows, wrows)
        return pltpu.make_async_copy(
            w_hbm[m].at[sl, :], stage_s.at[m, sl, :], w_sems.at[m * wparts + part]
        )

    for c in in_copies:
        c.start()
    for m in range(4):
        for part in range(wparts):
            w_copy(m, part).start()
    for c in in_copies:
        c.wait()

    kpad_s[0:8, :] = jnp.zeros((8, LANES), F32)
    sub = lax.broadcasted_iota(I32, (half, LANES), 0)
    sign = jnp.where((sub & 1) == 0, 1.0, -1.0).astype(F32)

    def conv_block(j, carry):
        ch = pl.ds(pl.multiple_of(j * LANES, LANES), LANES)
        fwd = fwd_ref[...]

        prev = None
        for a in range(nchunk):
            spec = lax.dot_general(
                fwd, ssm_s[ch, a * CHUNK:(a + 1) * CHUNK], _NT,
                preferred_element_type=F32)
            re, im = spec[:half], spec[half:]
            if prev is None:
                kf_s[a, 0:half, :] = re
                kf_s[a, half:, :] = im
            else:
                kf_s[a, 0:half, :] = re - sign * prev[1]
                kf_s[a, half:, :] = im + sign * prev[0]
            prev = (re, im)

        kpad_s[8:, :] = k_s[:, ch].astype(F32)
        taps = shift_ref[:, ch].astype(F32)
        for a in range(nchunk):
            acc = kpad_s[pl.ds(8 + a * CHUNK, CHUNK), :] * taps[0:1, :]
            for lag in range(1, taps.shape[0]):
                acc = acc + (
                    kpad_s[pl.ds(8 + a * CHUNK - lag, CHUNK), :] * taps[lag:lag + 1, :])
            kv = (acc * v_s[a * CHUNK:(a + 1) * CHUNK, ch].astype(F32)).astype(BF16)
            kv_s[a * CHUNK:(a + 1) * CHUNK, :] = kv
            xf_s[a] = jnp.dot(fwd, kv, preferred_element_type=F32)

        def freq_rows(i, c2):
            re_rows = pl.ds(pl.multiple_of(i * 8, 8), 8)
            im_rows = pl.ds(pl.multiple_of(half + i * 8, 8), 8)
            xr = [xf_s[a, re_rows, :] for a in range(nchunk)]
            xi = [xf_s[a, im_rows, :] for a in range(nchunk)]
            for c in range(nchunk):
                zr = zi = None
                for a in range(c + 1):
                    kr = kf_s[c - a, re_rows, :]
                    ki = kf_s[c - a, im_rows, :]
                    tr = xr[a] * kr - xi[a] * ki
                    ti = xr[a] * ki + xi[a] * kr
                    zr = tr if zr is None else zr + tr
                    zi = ti if zi is None else zi + ti
                zf_s[c, re_rows, :] = zr
                zf_s[c, im_rows, :] = zi
            return c2

        lax.fori_loop(0, half // 8, freq_rows, 0)

        inv = inv_ref[...]
        skip = ssmd_ref[:, ch].astype(F32)
        for c in range(nchunk):
            t = slice(c * CHUNK, (c + 1) * CHUNK)
            y = jnp.dot(inv, zf_s[c].astype(BF16), preferred_element_type=F32)
            y = y + kv_s[t, :].astype(F32) * skip
            b_s[t, ch] = x_s[t, ch].astype(F32) * y
        return carry

    lax.fori_loop(0, nblk, conv_block, 0)

    pairs_per_part = pairs // wparts
    for m in range(3):
        for part in range(wparts):
            w_copy(m, part).wait()

            def transpose_pair(i, carry, m=m, part=part):
                g = part * pairs_per_part + i
                src = stage_s[m, pl.ds(pl.multiple_of(g * pw, pw), pw), :]
                dst = pl.ds(pl.multiple_of((3 * g + m) * pw, LANES), pw)
                wqkv_s[:, dst] = pltpu.bitcast(src.T, I32)
                return carry

            lax.fori_loop(0, pairs_per_part, transpose_pair, 0)
    for part in range(wparts):
        w_copy(3, part).wait()

        def repack_pair(i, carry, part=part):
            g = part * pairs_per_part + i
            src = stage_s[3, pl.ds(pl.multiple_of(g * pw, pw), pw), :]
            wo_s[pl.ds(pl.multiple_of(g * dh, dh), dh), :] = pltpu.bitcast(src, I32)
            return carry

        lax.fori_loop(0, pairs_per_part, repack_pair, 0)

    scale = dh ** -0.5
    lane = lax.broadcasted_iota(I32, (rows, LANES), 1)
    first_half = lane < (dh - LANES)
    col = lax.broadcasted_iota(I32, (rows, 2 * rows), 1)
    row = lax.broadcasted_iota(I32, (rows, 2 * rows), 0)
    head0 = col < rows
    allowed = (row < nmem) | (row >= jnp.where(head0, col, col - rows))
    zeros = jnp.zeros((rows, LANES), F32)
    gate_w = gate_ref[...].astype(F32)

    def block_diag(t):
        a, b, c = t[:, :LANES], t[:, LANES:2 * LANES], t[:, 2 * LANES:]
        top = jnp.concatenate([a, jnp.where(first_half, b, 0.0), zeros], axis=1)
        bot = jnp.concatenate([zeros, jnp.where(first_half, 0.0, b), c], axis=1)
        return pltpu.bitcast(jnp.concatenate([top, bot], axis=0).astype(BF16), I32)

    def project(g):
        w = pltpu.bitcast(wqkv_s[:, 3 * g * pw:3 * (g + 1) * pw], BF16)
        qkv = jnp.dot(h_s[...], w, preferred_element_type=F32)
        q_s[g] = qkv[:, :pw]
        kb_s[g] = block_diag(qkv[:, pw:2 * pw])
        vb_s[g] = block_diag(qkv[:, 2 * pw:])

    def scores(g):
        s = lax.dot_general(
            q_s[g], pltpu.bitcast(kb_s[g], BF16), _NT, preferred_element_type=F32)
        s = jnp.where(allowed, s * scale, -1000000000.0)
        m0 = jnp.max(jnp.where(head0, s, -jnp.inf), axis=1, keepdims=True)
        m1 = jnp.max(jnp.where(head0, -jnp.inf, s), axis=1, keepdims=True)
        e = jnp.exp(s - jnp.where(head0, m0, m1))
        d0 = jnp.sum(jnp.where(head0, e, 0.0), axis=1, keepdims=True)
        d1 = jnp.sum(jnp.where(head0, 0.0, e), axis=1, keepdims=True)
        p_s[g] = e / jnp.where(head0, d0, d1)

    def values(g):
        o_s[:, g * pw:(g + 1) * pw] = jnp.dot(
            p_s[g], pltpu.bitcast(vb_s[g], BF16), preferred_element_type=F32)

    def out_proj(g0, g1):
        w = pltpu.bitcast(wo_s[g0 * dh:g1 * dh, :], BF16)
        return jnp.dot(o_s[:, g0 * pw:g1 * pw], w, preferred_element_type=F32)

    h_s[0:nmem, :] = mem0_ref[...].astype(F32)

    def segment(s, carry):
        t = pl.ds(pl.multiple_of(s * seg, seg), seg)
        xs = x_s[t, :].astype(F32)
        h_s[nmem:, :] = xs
        for g in range(pairs):
            project(g)
            if g >= 2:
                values(g - 2)
            if g >= 1:
                scores(g - 1)
        a = out_proj(0, pairs // 4)
        values(pairs - 2)
        scores(pairs - 1)
        a = a + out_proj(pairs // 4, pairs // 2)
        values(pairs - 1)
        a = a + out_proj(pairs // 2, pairs)
        h_s[0:nmem, :] = a[:nmem]
        gate = jax.nn.sigmoid(jnp.sum(xs * gate_w, axis=1, keepdims=True))
        out_s[t, :] = (gate * a[nmem:] + (1.0 - gate) * b_s[t, :]).astype(BF16)
        pltpu.make_async_copy(out_s.at[t, :], out_hbm.at[t, :], out_sem).start()
        return carry

    lax.fori_loop(0, nseg, segment, 0)
    pltpu.make_async_copy(out_s, out_hbm, out_sem).wait()


@functools.partial(jax.jit, static_argnames=("A_seg_len",))
def pallas_gated_mix__memory_aug_recurrent_mem_tr__ssm_conv_h3__prompt_kernel(
    A_x: jax.Array,
    A_mem0: jax.Array,
    A_Wq: jax.Array,
    A_Wk: jax.Array,
    A_Wv: jax.Array,
    A_Wo: jax.Array,
    A_seg_len: int,
    B_q: jax.Array,
    B_k: jax.Array,
    B_v: jax.Array,
    B_shift_k: jax.Array,
    B_ssm_k: jax.Array,
    B_ssm_D: jax.Array,
    gate_w: jax.Array,
):
    del B_q
    batch, seq, dm = A_x.shape
    _, heads, dh = A_Wq.shape
    nmem = A_mem0.shape[1]
    seg = int(A_seg_len)
    feat = heads * dh
    rows = nmem + seg
    pairs = heads // 2
    pw = 2 * dh
    nchunk = seq // CHUNK
    assert batch == 1 and dh == 192 and heads % 8 == 0 and dm % LANES == 0
    assert nmem % 8 == 0 and seg % 16 == 0 and seq % seg == 0 and 2 * rows <= LANES
    assert seq % CHUNK == 0 and B_shift_k.shape[1] <= 8

    def feature_major(w):
        return w.transpose(1, 2, 0).reshape(feat, dm)

    vmem = pl.BlockSpec(memory_space=pltpu.VMEM)
    hbm = pl.BlockSpec(memory_space=pltpu.HBM)
    out = pl.pallas_call(
        functools.partial(
            _kernel, seq=seq, dm=dm, heads=heads, dh=dh, nmem=nmem, seg=seg),
        out_shape=jax.ShapeDtypeStruct((seq, dm), BF16),
        in_specs=[vmem] * 6 + [hbm] * 8,
        out_specs=hbm,
        scratch_shapes=[
            pltpu.VMEM((seq, dm), BF16),
            pltpu.VMEM((seq, dm), BF16),
            pltpu.VMEM((seq, dm), BF16),
            pltpu.VMEM((dm, seq), BF16),
            pltpu.VMEM((4, feat, dm), BF16),
            pltpu.VMEM((dm // 2, 3 * feat), I32),
            pltpu.VMEM((feat // 2, dm), I32),
            pltpu.VMEM((8 + seq, LANES), F32),
            pltpu.VMEM((seq, LANES), BF16),
            pltpu.VMEM((nchunk, 2 * CHUNK, LANES), F32),
            pltpu.VMEM((nchunk, 2 * CHUNK, LANES), F32),
            pltpu.VMEM((nchunk, 2 * CHUNK, LANES), F32),
            pltpu.VMEM((seq, dm), F32),
            pltpu.VMEM((rows, dm), F32),
            pltpu.VMEM((pairs, rows, pw), F32),
            pltpu.VMEM((pairs, rows, pw), I32),
            pltpu.VMEM((pairs, rows, pw), I32),
            pltpu.VMEM((pairs, rows, 2 * rows), F32),
            pltpu.VMEM((rows, feat), F32),
            pltpu.VMEM((seq, dm), BF16),
            pltpu.SemaphoreType.DMA((4,)),
            pltpu.SemaphoreType.DMA((16,)),
            pltpu.SemaphoreType.DMA,
        ],
        compiler_params=pltpu.CompilerParams(vmem_limit_bytes=112 * 1024 * 1024),
        name="gated_mix_mem_h3",
    )(
        A_mem0.reshape(nmem, dm),
        B_shift_k.T,
        B_ssm_D.reshape(1, dm),
        gate_w.reshape(1, dm),
        jnp.asarray(_FWD, BF16),
        jnp.asarray(_INV, BF16),
        A_x.reshape(seq, dm),
        B_k.reshape(seq, dm),
        B_v.reshape(seq, dm),
        B_ssm_k,
        feature_major(A_Wq),
        feature_major(A_Wk),
        feature_major(A_Wv),
        A_Wo.reshape(feat, dm),
    )
    return out.reshape(batch, seq, dm)
```

```python
import functools

import jax
import jax.experimental.pallas as pl
import jax.experimental.pallas.tpu as pltpu
import jax.numpy as jnp
import numpy as np
from jax import lax

F32 = jnp.float32
BF16 = jnp.bfloat16
I32 = jnp.int32
LANES = 128
CHUNK = 128


def _dft_matrices(c):
    theta = np.pi * (np.arange(c)[:, None] + 0.5) * np.arange(c)[None, :] / c
    fwd = np.concatenate([np.cos(theta), -np.sin(theta)], axis=0)
    inv = np.concatenate([np.cos(theta).T, -np.sin(theta).T], axis=1) / c
    return fwd.astype(np.float32), inv.astype(np.float32)


_FWD, _INV = _dft_matrices(CHUNK)
_NT = (((1,), (1,)), ((), ()))


def _kernel(
    mem0_ref, shift_ref, ssmd_ref, gate_ref, fwd_ref, inv_ref,
    x_hbm, k_hbm, v_hbm, ssm_hbm, wq_hbm, wk_hbm, wv_hbm, wo_hbm,
    out_hbm,
    x_s, k_s, v_s, ssm_s, stage_s, wqkv_s, wo_s,
    kpad_s, kv_s, xf_s, kf_s, zf_s, b_s,
    h_s, q_s, kb_s, vb_s, p_s, o_s, out_s,
    in_sems, w_sems, out_sem,
    *, seq, dm, heads, dh, nmem, seg,
):
    feat = heads * dh
    rows = nmem + seg
    nseg = seq // seg
    pairs = heads // 2
    pw = 2 * dh
    nchunk = seq // CHUNK
    nblk = dm // LANES
    half = CHUNK
    wparts = 4
    wrows = feat // wparts
    w_hbm = (wq_hbm, wk_hbm, wv_hbm, wo_hbm)

    in_copies = [
        pltpu.make_async_copy(src, dst, in_sems.at[i])
        for i, (src, dst) in enumerate(
            ((ssm_hbm, ssm_s), (k_hbm, k_s), (v_hbm, v_s), (x_hbm, x_s))
        )
    ]

    def w_copy(m, part):
        sl = pl.ds(part * wrows, wrows)
        return pltpu.make_async_copy(
            w_hbm[m].at[sl, :], stage_s.at[m, sl, :], w_sems.at[m * wparts + part]
        )

    def start_weights(lo, hi):
        for i in range(lo, min(hi, 4 * wparts)):
            w_copy(i // wparts, i % wparts).start()

    for c in in_copies:
        c.start()
    for c in in_copies:
        c.wait()
    start_weights(0, 3)

    kpad_s[0:8, :] = jnp.zeros((8, LANES), F32)
    sub = lax.broadcasted_iota(I32, (half, LANES), 0)
    sign = jnp.where((sub & 1) == 0, 1.0, -1.0).astype(F32)

    def conv_block(j, carry):
        ch = pl.ds(pl.multiple_of(j * LANES, LANES), LANES)
        fwd = fwd_ref[...]

        prev = None
        for a in range(nchunk):
            spec = lax.dot_general(
                fwd, ssm_s[ch, a * CHUNK:(a + 1) * CHUNK], _NT,
                preferred_element_type=F32)
            re, im = spec[:half], spec[half:]
            if prev is None:
                kf_s[a, 0:half, :] = re
                kf_s[a, half:, :] = im
            else:
                kf_s[a, 0:half, :] = re - sign * prev[1]
                kf_s[a, half:, :] = im + sign * prev[0]
            prev = (re, im)

        kpad_s[8:, :] = k_s[:, ch].astype(F32)
        taps = shift_ref[:, ch].astype(F32)
        for a in range(nchunk):
            acc = kpad_s[pl.ds(8 + a * CHUNK, CHUNK), :] * taps[0:1, :]
            for lag in range(1, taps.shape[0]):
                acc = acc + (
                    kpad_s[pl.ds(8 + a * CHUNK - lag, CHUNK), :] * taps[lag:lag + 1, :])
            kv = (acc * v_s[a * CHUNK:(a + 1) * CHUNK, ch].astype(F32)).astype(BF16)
            kv_s[a * CHUNK:(a + 1) * CHUNK, :] = kv
            xf_s[a] = jnp.dot(fwd, kv, preferred_element_type=F32)

        def freq_rows(i, c2):
            re_rows = pl.ds(pl.multiple_of(i * 8, 8), 8)
            im_rows = pl.ds(pl.multiple_of(half + i * 8, 8), 8)
            xr = [xf_s[a, re_rows, :] for a in range(nchunk)]
            xi = [xf_s[a, im_rows, :] for a in range(nchunk)]
            for c in range(nchunk):
                zr = zi = None
                for a in range(c + 1):
                    kr = kf_s[c - a, re_rows, :]
                    ki = kf_s[c - a, im_rows, :]
                    tr = xr[a] * kr - xi[a] * ki
                    ti = xr[a] * ki + xi[a] * kr
                    zr = tr if zr is None else zr + tr
                    zi = ti if zi is None else zi + ti
                zf_s[c, re_rows, :] = zr
                zf_s[c, im_rows, :] = zi
            return c2

        lax.fori_loop(0, half // 8, freq_rows, 0)

        inv = inv_ref[...]
        skip = ssmd_ref[:, ch].astype(F32)
        for c in range(nchunk):
            t = slice(c * CHUNK, (c + 1) * CHUNK)
            y = jnp.dot(inv, zf_s[c].astype(BF16), preferred_element_type=F32)
            y = y + kv_s[t, :].astype(F32) * skip
            b_s[t, ch] = x_s[t, ch].astype(F32) * y
        for jj in range(nblk):
            pl.when(j == jj)(functools.partial(start_weights, 3 + 2 * jj, 5 + 2 * jj))
        return carry

    lax.fori_loop(0, nblk, conv_block, 0)
    start_weights(3 + 2 * nblk, 4 * wparts)

    pairs_per_part = pairs // wparts
    for m in range(3):
        for part in range(wparts):
            w_copy(m, part).wait()

            def transpose_pair(i, carry, m=m, part=part):
                g = part * pairs_per_part + i
                src = stage_s[m, pl.ds(pl.multiple_of(g * pw, pw), pw), :]
                dst = pl.ds(pl.multiple_of((3 * g + m) * pw, LANES), pw)
                wqkv_s[:, dst] = pltpu.bitcast(src.T, I32)
                return carry

            lax.fori_loop(0, pairs_per_part, transpose_pair, 0)
    for part in range(wparts):
        w_copy(3, part).wait()

        def repack_pair(i, carry, part=part):
            g = part * pairs_per_part + i
            src = stage_s[3, pl.ds(pl.multiple_of(g * pw, pw), pw), :]
            wo_s[pl.ds(pl.multiple_of(g * dh, dh), dh), :] = pltpu.bitcast(src, I32)
            return carry

        lax.fori_loop(0, pairs_per_part, repack_pair, 0)

    scale = dh ** -0.5
    lane = lax.broadcasted_iota(I32, (rows, LANES), 1)
    first_half = lane < (dh - LANES)
    col = lax.broadcasted_iota(I32, (rows, 2 * rows), 1)
    row = lax.broadcasted_iota(I32, (rows, 2 * rows), 0)
    head0 = col < rows
    allowed = (row < nmem) | (row >= jnp.where(head0, col, col - rows))
    zeros = jnp.zeros((rows, LANES), F32)
    gate_w = gate_ref[...].astype(F32)

    def block_diag(t):
        a, b, c = t[:, :LANES], t[:, LANES:2 * LANES], t[:, 2 * LANES:]
        top = jnp.concatenate([a, jnp.where(first_half, b, 0.0), zeros], axis=1)
        bot = jnp.concatenate([zeros, jnp.where(first_half, 0.0, b), c], axis=1)
        return pltpu.bitcast(jnp.concatenate([top, bot], axis=0).astype(BF16), I32)

    def project(g):
        w = pltpu.bitcast(wqkv_s[:, 3 * g * pw:3 * (g + 1) * pw], BF16)
        qkv = jnp.dot(h_s[...], w, preferred_element_type=F32)
        q_s[g] = qkv[:, :pw]
        kb_s[g] = block_diag(qkv[:, pw:2 * pw])
        vb_s[g] = block_diag(qkv[:, 2 * pw:])

    def scores(g):
        s = lax.dot_general(
            q_s[g], pltpu.bitcast(kb_s[g], BF16), _NT, preferred_element_type=F32)
        s = jnp.where(allowed, s * scale, -1000000000.0)
        m0 = jnp.max(jnp.where(head0, s, -jnp.inf), axis=1, keepdims=True)
        m1 = jnp.max(jnp.where(head0, -jnp.inf, s), axis=1, keepdims=True)
        e = jnp.exp(s - jnp.where(head0, m0, m1))
        d0 = jnp.sum(jnp.where(head0, e, 0.0), axis=1, keepdims=True)
        d1 = jnp.sum(jnp.where(head0, 0.0, e), axis=1, keepdims=True)
        p_s[g] = e / jnp.where(head0, d0, d1)

    def values(g):
        o_s[:, g * pw:(g + 1) * pw] = jnp.dot(
            p_s[g], pltpu.bitcast(vb_s[g], BF16), preferred_element_type=F32)

    def out_proj(g0, g1):
        w = pltpu.bitcast(wo_s[g0 * dh:g1 * dh, :], BF16)
        return jnp.dot(o_s[:, g0 * pw:g1 * pw], w, preferred_element_type=F32)

    h_s[0:nmem, :] = mem0_ref[...].astype(F32)

    def segment(s, carry):
        t = pl.ds(pl.multiple_of(s * seg, seg), seg)
        xs = x_s[t, :].astype(F32)
        h_s[nmem:, :] = xs
        for g in range(pairs):
            project(g)
            if g >= 2:
                values(g - 2)
            if g >= 1:
                scores(g - 1)
        a = out_proj(0, pairs // 4)
        values(pairs - 2)
        scores(pairs - 1)
        a = a + out_proj(pairs // 4, pairs // 2)
        values(pairs - 1)
        a = a + out_proj(pairs // 2, pairs)
        h_s[0:nmem, :] = a[:nmem]
        gate = jax.nn.sigmoid(jnp.sum(xs * gate_w, axis=1, keepdims=True))
        out_s[t, :] = (gate * a[nmem:] + (1.0 - gate) * b_s[t, :]).astype(BF16)
        pltpu.make_async_copy(out_s.at[t, :], out_hbm.at[t, :], out_sem).start()
        return carry

    lax.fori_loop(0, nseg, segment, 0)
    pltpu.make_async_copy(out_s, out_hbm, out_sem).wait()


@functools.partial(jax.jit, static_argnames=("A_seg_len",))
def pallas_gated_mix__memory_aug_recurrent_mem_tr__ssm_conv_h3__prompt_kernel(
    A_x: jax.Array,
    A_mem0: jax.Array,
    A_Wq: jax.Array,
    A_Wk: jax.Array,
    A_Wv: jax.Array,
    A_Wo: jax.Array,
    A_seg_len: int,
    B_q: jax.Array,
    B_k: jax.Array,
    B_v: jax.Array,
    B_shift_k: jax.Array,
    B_ssm_k: jax.Array,
    B_ssm_D: jax.Array,
    gate_w: jax.Array,
):
    del B_q
    batch, seq, dm = A_x.shape
    _, heads, dh = A_Wq.shape
    nmem = A_mem0.shape[1]
    seg = int(A_seg_len)
    feat = heads * dh
    rows = nmem + seg
    pairs = heads // 2
    pw = 2 * dh
    nchunk = seq // CHUNK
    assert batch == 1 and dh == 192 and heads % 8 == 0 and dm % LANES == 0
    assert nmem % 8 == 0 and seg % 16 == 0 and seq % seg == 0 and 2 * rows <= LANES
    assert seq % CHUNK == 0 and B_shift_k.shape[1] <= 8

    def feature_major(w):
        return w.transpose(1, 2, 0).reshape(feat, dm)

    vmem = pl.BlockSpec(memory_space=pltpu.VMEM)
    hbm = pl.BlockSpec(memory_space=pltpu.HBM)
    out = pl.pallas_call(
        functools.partial(
            _kernel, seq=seq, dm=dm, heads=heads, dh=dh, nmem=nmem, seg=seg),
        out_shape=jax.ShapeDtypeStruct((seq, dm), BF16),
        in_specs=[vmem] * 6 + [hbm] * 8,
        out_specs=hbm,
        scratch_shapes=[
            pltpu.VMEM((seq, dm), BF16),
            pltpu.VMEM((seq, dm), BF16),
            pltpu.VMEM((seq, dm), BF16),
            pltpu.VMEM((dm, seq), BF16),
            pltpu.VMEM((4, feat, dm), BF16),
            pltpu.VMEM((dm // 2, 3 * feat), I32),
            pltpu.VMEM((feat // 2, dm), I32),
            pltpu.VMEM((8 + seq, LANES), F32),
            pltpu.VMEM((seq, LANES), BF16),
            pltpu.VMEM((nchunk, 2 * CHUNK, LANES), F32),
            pltpu.VMEM((nchunk, 2 * CHUNK, LANES), F32),
            pltpu.VMEM((nchunk, 2 * CHUNK, LANES), F32),
            pltpu.VMEM((seq, dm), F32),
            pltpu.VMEM((rows, dm), F32),
            pltpu.VMEM((pairs, rows, pw), F32),
            pltpu.VMEM((pairs, rows, pw), I32),
            pltpu.VMEM((pairs, rows, pw), I32),
            pltpu.VMEM((pairs, rows, 2 * rows), F32),
            pltpu.VMEM((rows, feat), F32),
            pltpu.VMEM((seq, dm), BF16),
            pltpu.SemaphoreType.DMA((4,)),
            pltpu.SemaphoreType.DMA((16,)),
            pltpu.SemaphoreType.DMA,
        ],
        compiler_params=pltpu.CompilerParams(vmem_limit_bytes=112 * 1024 * 1024),
        name="gated_mix_mem_h3",
    )(
        A_mem0.reshape(nmem, dm),
        B_shift_k.T,
        B_ssm_D.reshape(1, dm),
        gate_w.reshape(1, dm),
        jnp.asarray(_FWD, BF16),
        jnp.asarray(_INV, BF16),
        A_x.reshape(seq, dm),
        B_k.reshape(seq, dm),
        B_v.reshape(seq, dm),
        B_ssm_k,
        feature_major(A_Wq),
        feature_major(A_Wk),
        feature_major(A_Wv),
        A_Wo.reshape(feat, dm),
    )
    return out.reshape(batch, seq, dm)
```

```python
import functools

import jax
import jax.experimental.pallas as pl
import jax.experimental.pallas.tpu as pltpu
import jax.numpy as jnp
import numpy as np
from jax import lax

F32 = jnp.float32
BF16 = jnp.bfloat16
I32 = jnp.int32
LANES = 128
CHUNK = 128


def _dft_matrices(c):
    theta = np.pi * (np.arange(c)[:, None] + 0.5) * np.arange(c)[None, :] / c
    fwd = np.concatenate([np.cos(theta), -np.sin(theta)], axis=0)
    inv = np.concatenate([np.cos(theta).T, -np.sin(theta).T], axis=1) / c
    return fwd.astype(np.float32), inv.astype(np.float32)


_FWD, _INV = _dft_matrices(CHUNK)
_NT = (((1,), (1,)), ((), ()))


def _kernel(
    mem0_ref, shift_ref, ssmd_ref, gate_ref, fwd_ref, inv_ref,
    x_hbm, k_hbm, v_hbm, ssm_hbm, wq_hbm, wk_hbm, wv_hbm, wo_hbm,
    out_hbm,
    x_s, k_s, v_s, ssm_s, stage_s, wqkv_s, wo_s,
    kpad_s, kv_s, xf_s, kf_s, zf_s, b_s,
    h_s, q_s, kb_s, vb_s, p_s, o_s, out_s,
    in_sems, w_sems, out_sem,
    *, seq, dm, heads, dh, nmem, seg,
):
    feat = heads * dh
    rows = nmem + seg
    nseg = seq // seg
    pairs = heads // 2
    pw = 2 * dh
    nchunk = seq // CHUNK
    nblk = dm // LANES
    half = CHUNK
    wparts = 4
    wrows = feat // wparts
    w_hbm = (wq_hbm, wk_hbm, wv_hbm, wo_hbm)

    in_copies = [
        pltpu.make_async_copy(src, dst, in_sems.at[i])
        for i, (src, dst) in enumerate(
            ((ssm_hbm, ssm_s), (k_hbm, k_s), (v_hbm, v_s), (x_hbm, x_s))
        )
    ]

    def w_copy(m, part):
        sl = pl.ds(part * wrows, wrows)
        return pltpu.make_async_copy(
            w_hbm[m].at[sl, :], stage_s.at[m, sl, :], w_sems.at[m * wparts + part]
        )

    def start_weights(lo, hi):
        for i in range(lo, min(hi, 4 * wparts)):
            w_copy(i // wparts, i % wparts).start()

    for c in in_copies:
        c.start()
    for c in in_copies:
        c.wait()
    start_weights(0, 3)

    kpad_s[0:8, :] = jnp.zeros((8, LANES), F32)
    sub = lax.broadcasted_iota(I32, (half, LANES), 0)
    sign = jnp.where((sub & 1) == 0, 1.0, -1.0).astype(F32)

    def conv_block(j, carry):
        ch = pl.ds(pl.multiple_of(j * LANES, LANES), LANES)
        fwd = fwd_ref[...]

        prev = None
        for a in range(nchunk):
            spec = lax.dot_general(
                fwd, ssm_s[ch, a * CHUNK:(a + 1) * CHUNK], _NT,
                preferred_element_type=F32)
            re, im = spec[:half], spec[half:]
            if prev is None:
                kf_s[a, 0:half, :] = re
                kf_s[a, half:, :] = im
            else:
                kf_s[a, 0:half, :] = re - sign * prev[1]
                kf_s[a, half:, :] = im + sign * prev[0]
            prev = (re, im)

        kpad_s[8:, :] = k_s[:, ch].astype(F32)
        taps = shift_ref[:, ch].astype(F32)
        for a in range(nchunk):
            acc = kpad_s[pl.ds(8 + a * CHUNK, CHUNK), :] * taps[0:1, :]
            for lag in range(1, taps.shape[0]):
                acc = acc + (
                    kpad_s[pl.ds(8 + a * CHUNK - lag, CHUNK), :] * taps[lag:lag + 1, :])
            kv = (acc * v_s[a * CHUNK:(a + 1) * CHUNK, ch].astype(F32)).astype(BF16)
            kv_s[a * CHUNK:(a + 1) * CHUNK, :] = kv
            xf_s[a] = jnp.dot(fwd, kv, preferred_element_type=F32)

        def freq_rows(i, c2):
            re_rows = pl.ds(pl.multiple_of(i * 8, 8), 8)
            im_rows = pl.ds(pl.multiple_of(half + i * 8, 8), 8)
            xr = [xf_s[a, re_rows, :] for a in range(nchunk)]
            xi = [xf_s[a, im_rows, :] for a in range(nchunk)]
            for c in range(nchunk):
                zr = zi = None
                for a in range(c + 1):
                    kr = kf_s[c - a, re_rows, :]
                    ki = kf_s[c - a, im_rows, :]
                    tr = xr[a] * kr - xi[a] * ki
                    ti = xr[a] * ki + xi[a] * kr
                    zr = tr if zr is None else zr + tr
                    zi = ti if zi is None else zi + ti
                zf_s[c, re_rows, :] = zr
                zf_s[c, im_rows, :] = zi
            return c2

        lax.fori_loop(0, half // 8, freq_rows, 0)

        inv = inv_ref[...]
        skip = ssmd_ref[:, ch].astype(F32)
        for c in range(nchunk):
            t = slice(c * CHUNK, (c + 1) * CHUNK)
            y = jnp.dot(inv, zf_s[c].astype(BF16), preferred_element_type=F32)
            y = y + kv_s[t, :].astype(F32) * skip
            b_s[t, ch] = x_s[t, ch].astype(F32) * y
        for jj in range(nblk):
            pl.when(j == jj)(functools.partial(start_weights, 3 + 2 * jj, 5 + 2 * jj))
        return carry

    lax.fori_loop(0, nblk, conv_block, 0)
    start_weights(3 + 2 * nblk, 4 * wparts)

    pairs_per_part = pairs // wparts
    for m in range(3):
        for part in range(wparts):
            w_copy(m, part).wait()

            def transpose_pair(i, carry, m=m, part=part):
                g = part * pairs_per_part + i
                src = stage_s[m, pl.ds(pl.multiple_of(g * pw, pw), pw), :]
                dst = pl.ds(pl.multiple_of((3 * g + m) * pw, LANES), pw)
                wqkv_s[:, dst] = pltpu.bitcast(src.T, I32)
                return carry

            lax.fori_loop(0, pairs_per_part, transpose_pair, 0)
    for part in range(wparts):
        w_copy(3, part).wait()

        def repack_pair(i, carry, part=part):
            g = part * pairs_per_part + i
            src = stage_s[3, pl.ds(pl.multiple_of(g * pw, pw), pw), :]
            wo_s[pl.ds(pl.multiple_of(g * dh, dh), dh), :] = pltpu.bitcast(src, I32)
            return carry

        lax.fori_loop(0, pairs_per_part, repack_pair, 0)

    scale = dh ** -0.5
    lane = lax.broadcasted_iota(I32, (rows, LANES), 1)
    first_half = lane < (dh - LANES)
    col = lax.broadcasted_iota(I32, (rows, 2 * rows), 1)
    row = lax.broadcasted_iota(I32, (rows, 2 * rows), 0)
    head0 = col < rows
    allowed = (row < nmem) | (row >= jnp.where(head0, col, col - rows))
    zeros = jnp.zeros((rows, LANES), F32)
    gate_w = gate_ref[...].astype(F32)

    def block_diag(t):
        a, b, c = t[:, :LANES], t[:, LANES:2 * LANES], t[:, 2 * LANES:]
        top = jnp.concatenate([a, jnp.where(first_half, b, 0.0), zeros], axis=1)
        bot = jnp.concatenate([zeros, jnp.where(first_half, 0.0, b), c], axis=1)
        return pltpu.bitcast(jnp.concatenate([top, bot], axis=0).astype(BF16), I32)

    def project(g):
        w = pltpu.bitcast(wqkv_s[:, 3 * g * pw:3 * (g + 1) * pw], BF16)
        qkv = jnp.dot(h_s[...], w, preferred_element_type=F32)
        q_s[g] = qkv[:, :pw]
        kb_s[g] = block_diag(qkv[:, pw:2 * pw])
        vb_s[g] = block_diag(qkv[:, 2 * pw:])

    def scores(g):
        s = lax.dot_general(
            q_s[g], pltpu.bitcast(kb_s[g], BF16), _NT, preferred_element_type=F32)
        s = jnp.where(allowed, s * scale, -1000000000.0)
        m0 = jnp.max(jnp.where(head0, s, -jnp.inf), axis=1, keepdims=True)
        m1 = jnp.max(jnp.where(head0, -jnp.inf, s), axis=1, keepdims=True)
        e = jnp.exp(s - jnp.where(head0, m0, m1))
        d0 = jnp.sum(jnp.where(head0, e, 0.0), axis=1, keepdims=True)
        d1 = jnp.sum(jnp.where(head0, 0.0, e), axis=1, keepdims=True)
        p_s[g] = e / jnp.where(head0, d0, d1)

    def values(g):
        o_s[:, g * pw:(g + 1) * pw] = jnp.dot(
            p_s[g], pltpu.bitcast(vb_s[g], BF16), preferred_element_type=F32)

    def out_proj(g0, g1):
        w = pltpu.bitcast(wo_s[g0 * dh:g1 * dh, :], BF16)
        return jnp.dot(o_s[:, g0 * pw:g1 * pw], w, preferred_element_type=F32)

    h_s[0:nmem, :] = mem0_ref[...].astype(F32)

    def segment(s, carry):
        t = pl.ds(pl.multiple_of(s * seg, seg), seg)
        xs = x_s[t, :].astype(F32)
        h_s[nmem:, :] = xs
        for g in range(pairs):
            project(g)
            if g >= 2:
                values(g - 2)
            if g >= 1:
                scores(g - 1)
        a = None
        for g in range(pairs):
            if g == 3:
                values(pairs - 2)
                scores(pairs - 1)
            if g == 6:
                values(pairs - 1)
            part = out_proj(g, g + 1)
            a = part if a is None else a + part
        h_s[0:nmem, :] = a[:nmem]
        gate = jax.nn.sigmoid(jnp.sum(xs * gate_w, axis=1, keepdims=True))
        out_s[t, :] = (gate * a[nmem:] + (1.0 - gate) * b_s[t, :]).astype(BF16)
        pltpu.make_async_copy(out_s.at[t, :], out_hbm.at[t, :], out_sem).start()
        return carry

    lax.fori_loop(0, nseg, segment, 0)
    pltpu.make_async_copy(out_s, out_hbm, out_sem).wait()


@functools.partial(jax.jit, static_argnames=("A_seg_len",))
def pallas_gated_mix__memory_aug_recurrent_mem_tr__ssm_conv_h3__prompt_kernel(
    A_x: jax.Array,
    A_mem0: jax.Array,
    A_Wq: jax.Array,
    A_Wk: jax.Array,
    A_Wv: jax.Array,
    A_Wo: jax.Array,
    A_seg_len: int,
    B_q: jax.Array,
    B_k: jax.Array,
    B_v: jax.Array,
    B_shift_k: jax.Array,
    B_ssm_k: jax.Array,
    B_ssm_D: jax.Array,
    gate_w: jax.Array,
):
    del B_q
    batch, seq, dm = A_x.shape
    _, heads, dh = A_Wq.shape
    nmem = A_mem0.shape[1]
    seg = int(A_seg_len)
    feat = heads * dh
    rows = nmem + seg
    pairs = heads // 2
    pw = 2 * dh
    nchunk = seq // CHUNK
    assert batch == 1 and dh == 192 and heads % 8 == 0 and dm % LANES == 0
    assert nmem % 8 == 0 and seg % 16 == 0 and seq % seg == 0 and 2 * rows <= LANES
    assert seq % CHUNK == 0 and B_shift_k.shape[1] <= 8

    def feature_major(w):
        return w.transpose(1, 2, 0).reshape(feat, dm)

    vmem = pl.BlockSpec(memory_space=pltpu.VMEM)
    hbm = pl.BlockSpec(memory_space=pltpu.HBM)
    out = pl.pallas_call(
        functools.partial(
            _kernel, seq=seq, dm=dm, heads=heads, dh=dh, nmem=nmem, seg=seg),
        out_shape=jax.ShapeDtypeStruct((seq, dm), BF16),
        in_specs=[vmem] * 6 + [hbm] * 8,
        out_specs=hbm,
        scratch_shapes=[
            pltpu.VMEM((seq, dm), BF16),
            pltpu.VMEM((seq, dm), BF16),
            pltpu.VMEM((seq, dm), BF16),
            pltpu.VMEM((dm, seq), BF16),
            pltpu.VMEM((4, feat, dm), BF16),
            pltpu.VMEM((dm // 2, 3 * feat), I32),
            pltpu.VMEM((feat // 2, dm), I32),
            pltpu.VMEM((8 + seq, LANES), F32),
            pltpu.VMEM((seq, LANES), BF16),
            pltpu.VMEM((nchunk, 2 * CHUNK, LANES), F32),
            pltpu.VMEM((nchunk, 2 * CHUNK, LANES), F32),
            pltpu.VMEM((nchunk, 2 * CHUNK, LANES), F32),
            pltpu.VMEM((seq, dm), F32),
            pltpu.VMEM((rows, dm), F32),
            pltpu.VMEM((pairs, rows, pw), F32),
            pltpu.VMEM((pairs, rows, pw), I32),
            pltpu.VMEM((pairs, rows, pw), I32),
            pltpu.VMEM((pairs, rows, 2 * rows), F32),
            pltpu.VMEM((rows, feat), F32),
            pltpu.VMEM((seq, dm), BF16),
            pltpu.SemaphoreType.DMA((4,)),
            pltpu.SemaphoreType.DMA((16,)),
            pltpu.SemaphoreType.DMA,
        ],
        compiler_params=pltpu.CompilerParams(vmem_limit_bytes=112 * 1024 * 1024),
        name="gated_mix_mem_h3",
    )(
        A_mem0.reshape(nmem, dm),
        B_shift_k.T,
        B_ssm_D.reshape(1, dm),
        gate_w.reshape(1, dm),
        jnp.asarray(_FWD, BF16),
        jnp.asarray(_INV, BF16),
        A_x.reshape(seq, dm),
        B_k.reshape(seq, dm),
        B_v.reshape(seq, dm),
        B_ssm_k,
        feature_major(A_Wq),
        feature_major(A_Wk),
        feature_major(A_Wv),
        A_Wo.reshape(feat, dm),
    )
    return out.reshape(batch, seq, dm)
```

```python
import functools

import jax
import jax.experimental.pallas as pl
import jax.experimental.pallas.tpu as pltpu
import jax.numpy as jnp
import numpy as np
from jax import lax

F32 = jnp.float32
BF16 = jnp.bfloat16
I32 = jnp.int32
LANES = 128
CHUNK = 128


def _dft_matrices(c):
    theta = np.pi * (np.arange(c)[:, None] + 0.5) * np.arange(c)[None, :] / c
    parts = np.stack([np.cos(theta), -np.sin(theta)])
    fwd = parts.reshape(2, c // 8, 8, c).transpose(1, 0, 2, 3).reshape(2 * c, c)
    return fwd.astype(np.float32), (fwd.T / c).astype(np.float32)


_FWD, _INV = _dft_matrices(CHUNK)
_NT = (((1,), (1,)), ((), ()))


def _interleave(*jobs):
    order = sorted(((i + 0.5) / n, j) for j, (_, n) in enumerate(jobs) for i in range(n))
    for _, j in order:
        next(jobs[j][0])
    for job, _ in jobs:
        for _ in job:
            pass


def _kernel(
    mem0_ref, shift_ref, ssmd_ref, gate_ref, fwd_ref, inv_ref,
    x_hbm, k_hbm, v_hbm, ssm_hbm, wq_hbm, wk_hbm, wv_hbm, wo_hbm,
    out_hbm,
    x_s, k_s, v_s, ssm_s, stage_s, wqkv_s, wo_s,
    kpad_s, xf_s, kf_s, zf_s, tail_s,
    h_s, q_s, kb_s, vb_s, p_s, o_s,
    in_sems, w_sems, out_sem,
    *, seq, dm, heads, dh, nmem, seg,
):
    rows = nmem + seg
    nseg = seq // seg
    pairs = heads // 2
    pw = 2 * dh
    nchunk = seq // CHUNK
    nblk = dm // LANES
    w_hbm = (wq_hbm, wk_hbm, wv_hbm)

    ssm_copies = [
        pltpu.make_async_copy(
            ssm_hbm.at[pl.ds(i * dm // 2, dm // 2), :],
            ssm_s.at[pl.ds(i * dm // 2, dm // 2), :], in_sems.at[i])
        for i in range(2)
    ]
    k_copy = pltpu.make_async_copy(k_hbm, k_s, in_sems.at[2])
    v_copy = pltpu.make_async_copy(v_hbm, v_s, in_sems.at[3])
    x_copy = pltpu.make_async_copy(x_hbm, x_s, in_sems.at[4])

    def w_copy(m, g):
        sl = pl.ds(pl.multiple_of(g * pw, pw), pw)
        if m == 3:
            return pltpu.make_async_copy(
                wo_hbm.at[sl, :], wo_s.at[sl, :], w_sems.at[m * pairs + g])
        return pltpu.make_async_copy(
            w_hbm[m].at[sl, :], stage_s.at[m, g], w_sems.at[m * pairs + g])

    def start_qkv(g):
        for m in range(3):
            w_copy(m, g).start()

    for c in ssm_copies:
        c.start()
    for c in ssm_copies:
        c.wait()
    k_copy.start()
    v_copy.start()

    sub = lax.broadcasted_iota(I32, (8, LANES), 0)
    sign = jnp.where((sub & 1) == 0, 1.0, -1.0).astype(F32)

    def filter_spectra(j, carry):
        ch = pl.ds(pl.multiple_of(j * LANES, LANES), LANES)
        fwd = fwd_ref[...]
        prev = None
        for a in range(nchunk):
            spec = lax.dot_general(
                fwd, ssm_s[ch, a * CHUNK:(a + 1) * CHUNK], _NT,
                preferred_element_type=F32).reshape(CHUNK // 8, 2, 8, LANES)
            if prev is None:
                folded = spec
            else:
                folded = jnp.stack(
                    [spec[:, 0] - sign * prev[:, 1], spec[:, 1] + sign * prev[:, 0]],
                    axis=1)
            kf_s[j, a] = folded.reshape(2 * CHUNK, LANES)
            prev = spec
        return carry

    lax.fori_loop(0, nblk, filter_spectra, 0)
    k_copy.wait()
    v_copy.wait()
    x_copy.start()
    start_qkv(0)
    kpad_s[0:8, :] = jnp.zeros((8, LANES), F32)

    def signal_spectra(j, carry):
        ch = pl.ds(pl.multiple_of(j * LANES, LANES), LANES)
        fwd = fwd_ref[...]
        kpad_s[8:, :] = k_s[:, ch].astype(F32)
        taps = shift_ref[:, ch].astype(F32)
        for a in range(nchunk):
            t = slice(a * CHUNK, (a + 1) * CHUNK)
            acc = kpad_s[pl.ds(8 + a * CHUNK, CHUNK), :] * taps[0:1, :]
            for lag in range(1, taps.shape[0]):
                acc = acc + (
                    kpad_s[pl.ds(8 + a * CHUNK - lag, CHUNK), :] * taps[lag:lag + 1, :])
            kv = (acc * v_s[t, ch].astype(F32)).astype(BF16)
            v_s[t, ch] = kv
            xf_s[j, a] = jnp.dot(fwd, kv, preferred_element_type=F32)
        pl.when(j == nblk // 2)(functools.partial(start_qkv, 1))
        return carry

    lax.fori_loop(0, nblk, signal_spectra, 0)
    x_copy.wait()

    for s in range(nseg):
        tail_s[8 * s:8 * s + 8, :] = (
            x_s[(s + 1) * seg - 16:(s + 1) * seg, :].astype(F32)[8:])

    tail_rows = 128

    def prepare(g, carry):
        for m in range(3):
            w_copy(m, g).wait()
        pl.when(g + 2 < pairs)(lambda: start_qkv(g + 2))
        w_copy(3, g).start()

        def tail_projection():
            for m in range(2):
                for n in range(pw // LANES):
                    w = stage_s[m, g, n * LANES:(n + 1) * LANES, :]
                    for r in range(0, 8 * nseg, tail_rows):
                        full = lax.dot_general(
                            tail_s[r:r + tail_rows, :], w, _NT, preferred_element_type=F32)
                        for i in range(0, tail_rows, 16):
                            word = (r + i) // 2
                            kf_s[nblk + 3 * m + n, g, word:word + 8, :] = pltpu.bitcast(
                                full[i:i + 16].astype(BF16), F32)
                            yield

        def transpose():
            for m in range(3):
                for n in range(pw // LANES):
                    w = stage_s[m, g, n * LANES:(n + 1) * LANES, :]
                    wqkv_s[g, :, m * pw + n * LANES:m * pw + (n + 1) * LANES] = (
                        pltpu.bitcast(w.T, I32))
                    yield

        def chunk_conv():
            re = pl.ds(pl.multiple_of(g * 16, 8), 8)
            im = pl.ds(pl.multiple_of(g * 16 + 8, 8), 8)
            for j in range(nblk):
                xr, xi = [], []
                for c in range(nchunk):
                    xr.append(xf_s[j, c, re, :])
                    xi.append(xf_s[j, c, im, :])
                    zr = zi = None
                    for a in range(c + 1):
                        kr = kf_s[j, c - a, re, :]
                        ki = kf_s[j, c - a, im, :]
                        tr = xr[a] * kr - xi[a] * ki
                        ti = xr[a] * ki + xi[a] * kr
                        zr = tr if zr is None else zr + tr
                        zi = ti if zi is None else zi + ti
                        yield
                    z = jnp.concatenate([zr, zi], axis=0).astype(BF16)
                    zf_s[j, c, pl.ds(pl.multiple_of(g * 8, 8), 8), :] = (
                        pltpu.bitcast(z, I32))

        _interleave(
            (tail_projection(), 2 * (pw // LANES) * nseg // 2),
            (chunk_conv(), nblk * nchunk * (nchunk + 1) // 2),
            (transpose(), 3 * (pw // LANES)),
        )
        return carry

    lax.fori_loop(0, pairs, prepare, 0)

    def finish_conv(j, carry):
        ch = pl.ds(pl.multiple_of(j * LANES, LANES), LANES)
        inv = inv_ref[...]
        skip = ssmd_ref[:, ch].astype(F32)
        for c in range(nchunk):
            t = slice(c * CHUNK, (c + 1) * CHUNK)
            y = jnp.dot(
                inv, pltpu.bitcast(zf_s[j, c], BF16), preferred_element_type=F32)
            y = y + v_s[t, ch].astype(F32) * skip
            kf_s[j, c, 0:CHUNK, :] = x_s[t, ch].astype(F32) * y
        return carry

    lax.fori_loop(0, nblk, finish_conv, 0)
    for g in range(pairs):
        w_copy(3, g).wait()

    scale = dh ** -0.5
    head = rows - 8
    lane = lax.broadcasted_iota(I32, (rows, LANES), 1)
    first_half = lane < (dh - LANES)
    col = lax.broadcasted_iota(I32, (rows, 2 * rows), 1)
    row = lax.broadcasted_iota(I32, (rows, 2 * rows), 0)
    head0 = col < rows
    allowed = (row < nmem) | (row >= jnp.where(head0, col, col - rows))
    zeros = jnp.zeros((rows, LANES), F32)
    gate_w = gate_ref[...].astype(F32)
    out_s = k_s

    def block_diag(t):
        a, b, c = t[:, :LANES], t[:, LANES:2 * LANES], t[:, 2 * LANES:]
        top = jnp.concatenate([a, jnp.where(first_half, b, 0.0), zeros], axis=1)
        bot = jnp.concatenate([zeros, jnp.where(first_half, 0.0, b), c], axis=1)
        return pltpu.bitcast(jnp.concatenate([top, bot], axis=0).astype(BF16), I32)

    def project(g, s):
        two = pl.ds(pl.multiple_of((s // 2) * 8, 8), 8)
        qk = []
        for m in range(2):
            w = pltpu.bitcast(wqkv_s[g, :, m * pw:(m + 1) * pw], BF16)
            most = jnp.dot(h_s[0:head, :], w, preferred_element_type=F32)
            words = [kf_s[nblk + 3 * m + n, g, two, :] for n in range(pw // LANES)]
            both = pltpu.bitcast(jnp.concatenate(words, axis=1), BF16).astype(F32)
            tail = jnp.where(s % 2 == 0, both[:8], both[8:])
            qk.append(jnp.concatenate([most, tail], axis=0))
        q_s[g] = qk[0]
        kb_s[g] = block_diag(qk[1])
        w = pltpu.bitcast(wqkv_s[g, :, 2 * pw:], BF16)
        vb_s[g] = block_diag(jnp.dot(h_s[...], w, preferred_element_type=F32))

    def scores(g):
        s = lax.dot_general(
            q_s[g], pltpu.bitcast(kb_s[g], BF16), _NT, preferred_element_type=F32)
        s = jnp.where(allowed, s * scale, -1000000000.0)
        m0 = jnp.max(jnp.where(head0, s, -jnp.inf), axis=1, keepdims=True)
        m1 = jnp.max(jnp.where(head0, -jnp.inf, s), axis=1, keepdims=True)
        e = jnp.exp(s - jnp.where(head0, m0, m1))
        d0 = jnp.sum(jnp.where(head0, e, 0.0), axis=1, keepdims=True)
        d1 = jnp.sum(jnp.where(head0, 0.0, e), axis=1, keepdims=True)
        p_s[g] = e / jnp.where(head0, d0, d1)

    def values(g):
        o_s[:, g * pw:(g + 1) * pw] = jnp.dot(
            p_s[g], pltpu.bitcast(vb_s[g], BF16), preferred_element_type=F32)

    def out_proj(g):
        return jnp.dot(
            o_s[:, g * pw:(g + 1) * pw], wo_s[g * pw:(g + 1) * pw, :],
            preferred_element_type=F32)

    h_s[0:nmem, :] = mem0_ref[...].astype(F32)

    def segment(s, carry):
        t = pl.ds(pl.multiple_of(s * seg, seg), seg)
        xs = x_s[t, :].astype(F32)
        h_s[nmem:, :] = xs
        for g in range(pairs):
            project(g, s)
            if g >= 2:
                values(g - 2)
            if g >= 1:
                scores(g - 1)
        a = None
        for g in range(pairs):
            if g == 3:
                values(pairs - 2)
                scores(pairs - 1)
            if g == 6:
                values(pairs - 1)
            part = out_proj(g)
            a = part if a is None else a + part
        h_s[0:nmem, :] = a[:nmem]
        per_chunk = CHUNK // seg
        in_chunk = pl.ds(pl.multiple_of((s % per_chunk) * seg, seg), seg)
        b = jnp.concatenate(
            [kf_s[j, s // per_chunk, in_chunk, :] for j in range(nblk)], axis=1)
        gate = jax.nn.sigmoid(jnp.sum(xs * gate_w, axis=1, keepdims=True))
        out_s[t, :] = (gate * a[nmem:] + (1.0 - gate) * b).astype(BF16)
        pltpu.make_async_copy(out_s.at[t, :], out_hbm.at[t, :], out_sem).start()
        return carry

    lax.fori_loop(0, nseg, segment, 0)
    pltpu.make_async_copy(out_s, out_hbm, out_sem).wait()


@functools.partial(jax.jit, static_argnames=("A_seg_len",))
def pallas_gated_mix__memory_aug_recurrent_mem_tr__ssm_conv_h3__prompt_kernel(
    A_x: jax.Array,
    A_mem0: jax.Array,
    A_Wq: jax.Array,
    A_Wk: jax.Array,
    A_Wv: jax.Array,
    A_Wo: jax.Array,
    A_seg_len: int,
    B_q: jax.Array,
    B_k: jax.Array,
    B_v: jax.Array,
    B_shift_k: jax.Array,
    B_ssm_k: jax.Array,
    B_ssm_D: jax.Array,
    gate_w: jax.Array,
):
    del B_q
    batch, seq, dm = A_x.shape
    _, heads, dh = A_Wq.shape
    nmem = A_mem0.shape[1]
    seg = int(A_seg_len)
    feat = heads * dh
    rows = nmem + seg
    pairs = heads // 2
    pw = 2 * dh
    nchunk = seq // CHUNK
    nblk = dm // LANES
    nseg = seq // seg
    assert pairs == CHUNK // 8 and nseg % 2 == 0 and CHUNK % seg == 0
    assert batch == 1 and dh == 192 and heads % 8 == 0 and dm % LANES == 0
    assert nmem % 8 == 0 and seg % 16 == 0 and seq % seg == 0 and 2 * rows <= LANES
    assert seq % CHUNK == 0 and B_shift_k.shape[1] <= 8

    def feature_major(w):
        return w.transpose(1, 2, 0).reshape(feat, dm)

    vmem = pl.BlockSpec(memory_space=pltpu.VMEM)
    hbm = pl.BlockSpec(memory_space=pltpu.HBM)
    out = pl.pallas_call(
        functools.partial(
            _kernel, seq=seq, dm=dm, heads=heads, dh=dh, nmem=nmem, seg=seg),
        out_shape=jax.ShapeDtypeStruct((seq, dm), BF16),
        in_specs=[vmem] * 6 + [hbm] * 8,
        out_specs=hbm,
        scratch_shapes=[
            pltpu.VMEM((seq, dm), BF16),
            pltpu.VMEM((seq, dm), BF16),
            pltpu.VMEM((seq, dm), BF16),
            pltpu.VMEM((dm, seq), BF16),
            pltpu.VMEM((3, pairs, pw, dm), BF16),
            pltpu.VMEM((pairs, dm // 2, 3 * pw), I32),
            pltpu.VMEM((feat, dm), BF16),
            pltpu.VMEM((8 + seq, LANES), F32),
            pltpu.VMEM((nblk, nchunk, 2 * CHUNK, LANES), F32),
            pltpu.VMEM((nblk + 6, nchunk, 2 * CHUNK, LANES), F32),
            pltpu.VMEM((nblk, nchunk, CHUNK, LANES), I32),
            pltpu.VMEM((8 * nseg, dm), F32),
            pltpu.VMEM((rows, dm), F32),
            pltpu.VMEM((pairs, rows, pw), F32),
            pltpu.VMEM((pairs, rows, pw), I32),
            pltpu.VMEM((pairs, rows, pw), I32),
            pltpu.VMEM((pairs, rows, 2 * rows), F32),
            pltpu.VMEM((rows, feat), F32),
            pltpu.SemaphoreType.DMA((5,)),
            pltpu.SemaphoreType.DMA((4 * pairs,)),
            pltpu.SemaphoreType.DMA,
        ],
        compiler_params=pltpu.CompilerParams(vmem_limit_bytes=112 * 1024 * 1024),
        name="gated_mix_mem_h3",
    )(
        A_mem0.reshape(nmem, dm),
        B_shift_k.T,
        B_ssm_D.reshape(1, dm),
        gate_w.reshape(1, dm),
        jnp.asarray(_FWD, BF16),
        jnp.asarray(_INV, BF16),
        A_x.reshape(seq, dm),
        B_k.reshape(seq, dm),
        B_v.reshape(seq, dm),
        B_ssm_k,
        feature_major(A_Wq),
        feature_major(A_Wk),
        feature_major(A_Wv),
        A_Wo.reshape(feat, dm),
    )
    return out.reshape(batch, seq, dm)
```

```python
import functools

import jax
import jax.experimental.pallas as pl
import jax.experimental.pallas.tpu as pltpu
import jax.numpy as jnp
import numpy as np
from jax import lax

F32 = jnp.float32
BF16 = jnp.bfloat16
I32 = jnp.int32
LANES = 128
CHUNK = 128


def _dft_matrices(c):
    theta = np.pi * (np.arange(c)[:, None] + 0.5) * np.arange(c)[None, :] / c
    parts = np.stack([np.cos(theta), -np.sin(theta)])
    fwd = parts.reshape(2, c // 8, 8, c).transpose(1, 0, 2, 3).reshape(2 * c, c)
    return fwd.astype(np.float32), (fwd.T / c).astype(np.float32)


_FWD, _INV = _dft_matrices(CHUNK)
_NT = (((1,), (1,)), ((), ()))


def _interleave(*jobs):
    order = sorted(((i + 0.5) / n, j) for j, (_, n) in enumerate(jobs) for i in range(n))
    for _, j in order:
        next(jobs[j][0])
    for job, _ in jobs:
        for _ in job:
            pass


def _step_schedule(pairs):
    order = []
    for g in range(pairs):
        order += [("q", g), ("v", g), ("s", g - 1), ("k", g), ("o", g - 7), ("p", g - 2)]
    for op, back in zip("oospooopoo", (7, 6, 1, 2, 5, 4, 3, 1, 2, 1)):
        order.append((op, pairs - back))
    return [(op, g) for op, g in order if g >= 0]


def _kernel(
    mem0_ref, shift_ref, ssmd_ref, gate_ref, fwd_ref, inv_ref,
    x_hbm, k_hbm, v_hbm, ssm_hbm, wq_hbm, wk_hbm, wv_hbm, wo_hbm,
    out_hbm,
    x_s, k_s, v_s, ssm_s, stage_s, wqkv_s, wo_s,
    kpad_s, xf_s, kf_s, zf_s, tail_s,
    h_s, q_s, kb_s, vb_s, p_s, o_s,
    in_sems, w_sems, out_sem,
    *, seq, dm, heads, dh, nmem, seg,
):
    rows = nmem + seg
    nseg = seq // seg
    pairs = heads // 2
    pw = 2 * dh
    nchunk = seq // CHUNK
    nblk = dm // LANES
    w_hbm = (wq_hbm, wk_hbm, wv_hbm)

    ssm_copies = [
        pltpu.make_async_copy(
            ssm_hbm.at[pl.ds(i * dm // 2, dm // 2), :],
            ssm_s.at[pl.ds(i * dm // 2, dm // 2), :], in_sems.at[i])
        for i in range(2)
    ]
    k_copy = pltpu.make_async_copy(k_hbm, k_s, in_sems.at[2])
    v_copy = pltpu.make_async_copy(v_hbm, v_s, in_sems.at[3])
    x_copy = pltpu.make_async_copy(x_hbm, x_s, in_sems.at[4])

    def w_copy(m, g):
        sl = pl.ds(pl.multiple_of(g * pw, pw), pw)
        if m == 3:
            return pltpu.make_async_copy(
                wo_hbm.at[sl, :], wo_s.at[sl, :], w_sems.at[m * pairs + g])
        return pltpu.make_async_copy(
            w_hbm[m].at[sl, :], stage_s.at[m, g], w_sems.at[m * pairs + g])

    def start_qkv(g):
        for m in range(3):
            w_copy(m, g).start()

    for c in ssm_copies:
        c.start()
    for c in ssm_copies:
        c.wait()
    k_copy.start()
    v_copy.start()

    sub = lax.broadcasted_iota(I32, (8, LANES), 0)
    sign = jnp.where((sub & 1) == 0, 1.0, -1.0).astype(F32)

    def filter_spectra(j, carry):
        ch = pl.ds(pl.multiple_of(j * LANES, LANES), LANES)
        fwd = fwd_ref[...]
        prev = None
        for a in range(nchunk):
            spec = lax.dot_general(
                fwd, ssm_s[ch, a * CHUNK:(a + 1) * CHUNK], _NT,
                preferred_element_type=F32).reshape(CHUNK // 8, 2, 8, LANES)
            if prev is None:
                folded = spec
            else:
                folded = jnp.stack(
                    [spec[:, 0] - sign * prev[:, 1], spec[:, 1] + sign * prev[:, 0]],
                    axis=1)
            kf_s[j, a] = folded.reshape(2 * CHUNK, LANES)
            prev = spec
        return carry

    lax.fori_loop(0, nblk, filter_spectra, 0)
    k_copy.wait()
    v_copy.wait()
    x_copy.start()
    start_qkv(0)
    kpad_s[0:8, :] = jnp.zeros((8, LANES), F32)

    def signal_spectra(j, carry):
        ch = pl.ds(pl.multiple_of(j * LANES, LANES), LANES)
        fwd = fwd_ref[...]
        kpad_s[8:, :] = k_s[:, ch].astype(F32)
        taps = shift_ref[:, ch].astype(F32)
        for a in range(nchunk):
            t = slice(a * CHUNK, (a + 1) * CHUNK)
            acc = kpad_s[pl.ds(8 + a * CHUNK, CHUNK), :] * taps[0:1, :]
            for lag in range(1, taps.shape[0]):
                acc = acc + (
                    kpad_s[pl.ds(8 + a * CHUNK - lag, CHUNK), :] * taps[lag:lag + 1, :])
            kv = (acc * v_s[t, ch].astype(F32)).astype(BF16)
            v_s[t, ch] = kv
            xf_s[j, a] = jnp.dot(fwd, kv, preferred_element_type=F32)
        pl.when(j == nblk // 2)(functools.partial(start_qkv, 1))
        return carry

    lax.fori_loop(0, nblk, signal_spectra, 0)
    x_copy.wait()

    for s in range(nseg):
        tail_s[8 * s:8 * s + 8, :] = (
            x_s[(s + 1) * seg - 16:(s + 1) * seg, :].astype(F32)[8:])

    tail_rows = 128

    def prepare(g, carry):
        for m in range(3):
            w_copy(m, g).wait()
        pl.when(g + 2 < pairs)(lambda: start_qkv(g + 2))
        w_copy(3, g).start()

        last = [None]

        def tail_projection():
            for m in range(2):
                for n in range(pw // LANES):
                    w = stage_s[m, g, n * LANES:(n + 1) * LANES, :]
                    for r in range(0, 8 * nseg, tail_rows):
                        full = lax.dot_general(
                            tail_s[r:r + tail_rows, :], w, _NT, preferred_element_type=F32)
                        for i in range(0, tail_rows, 16):
                            word = (r + i) // 2
                            last[0] = pltpu.bitcast(full[i:i + 16].astype(BF16), F32)
                            kf_s[nblk + 3 * m + n, g, word:word + 8, :] = last[0]
                            yield

        def transpose():
            for m in range(3):
                for n in range(pw // LANES):
                    w = stage_s[m, g, n * LANES:(n + 1) * LANES, :]
                    wqkv_s[g, 0:dm // 2, m * pw + n * LANES:m * pw + (n + 1) * LANES] = (
                        pltpu.bitcast(w.T, I32))
                    wqkv_s[pairs - 1 - g, dm // 2:, 0:LANES] = pltpu.bitcast(last[0], I32)
                    yield

        def chunk_conv():
            re = pl.ds(pl.multiple_of(g * 16, 8), 8)
            im = pl.ds(pl.multiple_of(g * 16 + 8, 8), 8)
            for j in range(nblk):
                xr, xi = [], []
                for c in range(nchunk):
                    xr.append(xf_s[j, c, re, :])
                    xi.append(xf_s[j, c, im, :])
                    zr = zi = None
                    for a in range(c + 1):
                        kr = kf_s[j, c - a, re, :]
                        ki = kf_s[j, c - a, im, :]
                        tr = xr[a] * kr - xi[a] * ki
                        ti = xr[a] * ki + xi[a] * kr
                        zr = tr if zr is None else zr + tr
                        zi = ti if zi is None else zi + ti
                        yield
                    z = jnp.concatenate([zr, zi], axis=0).astype(BF16)
                    zf_s[j, c, pl.ds(pl.multiple_of(g * 8, 8), 8), :] = (
                        pltpu.bitcast(z, I32))

        _interleave(
            (tail_projection(), 2 * (pw // LANES) * nseg // 2),
            (chunk_conv(), nblk * nchunk * (nchunk + 1) // 2),
            (transpose(), 3 * (pw // LANES)),
        )
        return carry

    lax.fori_loop(0, pairs, prepare, 0)

    def finish_conv(j, carry):
        ch = pl.ds(pl.multiple_of(j * LANES, LANES), LANES)
        inv = inv_ref[...]
        skip = ssmd_ref[:, ch].astype(F32)
        for c in range(nchunk):
            t = slice(c * CHUNK, (c + 1) * CHUNK)
            y = jnp.dot(
                inv, pltpu.bitcast(zf_s[j, c], BF16), preferred_element_type=F32)
            y = y + v_s[t, ch].astype(F32) * skip
            kf_s[j, c, 0:CHUNK, :] = x_s[t, ch].astype(F32) * y
        return carry

    lax.fori_loop(0, nblk, finish_conv, 0)
    for g in range(pairs):
        w_copy(3, g).wait()

    scale = dh ** -0.5
    head = rows - 8
    lane = lax.broadcasted_iota(I32, (rows, LANES), 1)
    first_half = lane < (dh - LANES)
    col = lax.broadcasted_iota(I32, (rows, 2 * rows), 1)
    row = lax.broadcasted_iota(I32, (rows, 2 * rows), 0)
    head0 = col < rows
    allowed = (row < nmem) | (row >= jnp.where(head0, col, col - rows))
    zeros = jnp.zeros((rows, LANES), F32)
    gate_w = gate_ref[...].astype(F32)
    out_s = k_s

    def block_diag(t):
        a, b, c = t[:, :LANES], t[:, LANES:2 * LANES], t[:, 2 * LANES:]
        top = jnp.concatenate([a, jnp.where(first_half, b, 0.0), zeros], axis=1)
        bot = jnp.concatenate([zeros, jnp.where(first_half, 0.0, b), c], axis=1)
        return pltpu.bitcast(jnp.concatenate([top, bot], axis=0).astype(BF16), I32)

    def project_qk(m, g, s):
        two = pl.ds(pl.multiple_of((s // 2) * 8, 8), 8)
        w = pltpu.bitcast(wqkv_s[g, 0:dm // 2, m * pw:(m + 1) * pw], BF16)
        most = jnp.dot(h_s[0:head, :], w, preferred_element_type=F32)
        words = [kf_s[nblk + 3 * m + n, g, two, :] for n in range(pw // LANES)]
        both = pltpu.bitcast(jnp.concatenate(words, axis=1), BF16).astype(F32)
        tail = jnp.where(s % 2 == 0, both[:8], both[8:])
        return jnp.concatenate([most, tail], axis=0)

    def queries(g, s):
        q_s[g] = project_qk(0, g, s)

    def keys(g, s):
        kb_s[g] = block_diag(project_qk(1, g, s))

    def vals(g):
        w = pltpu.bitcast(wqkv_s[g, 0:dm // 2, 2 * pw:], BF16)
        vb_s[g] = block_diag(jnp.dot(h_s[...], w, preferred_element_type=F32))

    def scores(g):
        s = lax.dot_general(
            q_s[g], pltpu.bitcast(kb_s[g], BF16), _NT, preferred_element_type=F32)
        s = jnp.where(allowed, s * scale, -1000000000.0)
        m0 = jnp.max(jnp.where(head0, s, -jnp.inf), axis=1, keepdims=True)
        m1 = jnp.max(jnp.where(head0, -jnp.inf, s), axis=1, keepdims=True)
        e = jnp.exp(s - jnp.where(head0, m0, m1))
        d0 = jnp.sum(jnp.where(head0, e, 0.0), axis=1, keepdims=True)
        d1 = jnp.sum(jnp.where(head0, 0.0, e), axis=1, keepdims=True)
        p_s[g] = e / jnp.where(head0, d0, d1)

    def values(g):
        o_s[:, g * pw:(g + 1) * pw] = jnp.dot(
            p_s[g], pltpu.bitcast(vb_s[g], BF16), preferred_element_type=F32)

    def out_proj(g):
        return jnp.dot(
            o_s[:, g * pw:(g + 1) * pw], wo_s[g * pw:(g + 1) * pw, :],
            preferred_element_type=F32)

    h_s[0:nmem, :] = mem0_ref[...].astype(F32)

    def segment(s, carry):
        t = pl.ds(pl.multiple_of(s * seg, seg), seg)
        xs = x_s[t, :].astype(F32)
        h_s[nmem:, :] = xs
        a = None
        for op, g in _step_schedule(pairs):
            if op == "o":
                part = out_proj(g)
                a = part if a is None else a + part
            else:
                dict(q=lambda: queries(g, s), k=lambda: keys(g, s), v=lambda: vals(g),
                     s=lambda: scores(g), p=lambda: values(g))[op]()
        h_s[0:nmem, :] = a[:nmem]
        per_chunk = CHUNK // seg
        in_chunk = pl.ds(pl.multiple_of((s % per_chunk) * seg, seg), seg)
        b = jnp.concatenate(
            [kf_s[j, s // per_chunk, in_chunk, :] for j in range(nblk)], axis=1)
        gate = jax.nn.sigmoid(jnp.sum(xs * gate_w, axis=1, keepdims=True))
        out_s[t, :] = (gate * a[nmem:] + (1.0 - gate) * b).astype(BF16)
        pltpu.make_async_copy(out_s.at[t, :], out_hbm.at[t, :], out_sem).start()
        return carry

    lax.fori_loop(0, nseg, segment, 0)
    pltpu.make_async_copy(out_s, out_hbm, out_sem).wait()


@functools.partial(jax.jit, static_argnames=("A_seg_len",))
def pallas_gated_mix__memory_aug_recurrent_mem_tr__ssm_conv_h3__prompt_kernel(
    A_x: jax.Array,
    A_mem0: jax.Array,
    A_Wq: jax.Array,
    A_Wk: jax.Array,
    A_Wv: jax.Array,
    A_Wo: jax.Array,
    A_seg_len: int,
    B_q: jax.Array,
    B_k: jax.Array,
    B_v: jax.Array,
    B_shift_k: jax.Array,
    B_ssm_k: jax.Array,
    B_ssm_D: jax.Array,
    gate_w: jax.Array,
):
    del B_q
    batch, seq, dm = A_x.shape
    _, heads, dh = A_Wq.shape
    nmem = A_mem0.shape[1]
    seg = int(A_seg_len)
    feat = heads * dh
    rows = nmem + seg
    pairs = heads // 2
    pw = 2 * dh
    nchunk = seq // CHUNK
    nblk = dm // LANES
    nseg = seq // seg
    assert pairs == CHUNK // 8 and nseg % 2 == 0 and CHUNK % seg == 0
    assert batch == 1 and dh == 192 and heads % 8 == 0 and dm % LANES == 0
    assert nmem % 8 == 0 and seg % 16 == 0 and seq % seg == 0 and 2 * rows <= LANES
    assert seq % CHUNK == 0 and B_shift_k.shape[1] <= 8

    def feature_major(w):
        return w.transpose(1, 2, 0).reshape(feat, dm)

    vmem = pl.BlockSpec(memory_space=pltpu.VMEM)
    hbm = pl.BlockSpec(memory_space=pltpu.HBM)
    out = pl.pallas_call(
        functools.partial(
            _kernel, seq=seq, dm=dm, heads=heads, dh=dh, nmem=nmem, seg=seg),
        out_shape=jax.ShapeDtypeStruct((seq, dm), BF16),
        in_specs=[vmem] * 6 + [hbm] * 8,
        out_specs=hbm,
        scratch_shapes=[
            pltpu.VMEM((seq, dm), BF16),
            pltpu.VMEM((seq, dm), BF16),
            pltpu.VMEM((seq, dm), BF16),
            pltpu.VMEM((dm, seq), BF16),
            pltpu.VMEM((3, pairs, pw, dm), BF16),
            pltpu.VMEM((pairs, dm // 2 + 8, 3 * pw), I32),
            pltpu.VMEM((feat, dm), BF16),
            pltpu.VMEM((8 + seq, LANES), F32),
            pltpu.VMEM((nblk, nchunk, 2 * CHUNK, LANES), F32),
            pltpu.VMEM((nblk + 6, nchunk, 2 * CHUNK, LANES), F32),
            pltpu.VMEM((nblk, nchunk, CHUNK, LANES), I32),
            pltpu.VMEM((8 * nseg, dm), F32),
            pltpu.VMEM((rows, dm), F32),
            pltpu.VMEM((pairs, rows, pw), F32),
            pltpu.VMEM((pairs, rows, pw), I32),
            pltpu.VMEM((pairs, rows, pw), I32),
            pltpu.VMEM((pairs, rows, 2 * rows), F32),
            pltpu.VMEM((rows, feat), F32),
            pltpu.SemaphoreType.DMA((5,)),
            pltpu.SemaphoreType.DMA((4 * pairs,)),
            pltpu.SemaphoreType.DMA,
        ],
        compiler_params=pltpu.CompilerParams(vmem_limit_bytes=112 * 1024 * 1024),
        name="gated_mix_mem_h3",
    )(
        A_mem0.reshape(nmem, dm),
        B_shift_k.T,
        B_ssm_D.reshape(1, dm),
        gate_w.reshape(1, dm),
        jnp.asarray(_FWD, BF16),
        jnp.asarray(_INV, BF16),
        A_x.reshape(seq, dm),
        B_k.reshape(seq, dm),
        B_v.reshape(seq, dm),
        B_ssm_k,
        feature_major(A_Wq),
        feature_major(A_Wk),
        feature_major(A_Wv),
        A_Wo.reshape(feat, dm),
    )
    return out.reshape(batch, seq, dm)
```

```python
import functools

import jax
import jax.experimental.pallas as pl
import jax.experimental.pallas.tpu as pltpu
import jax.numpy as jnp
import numpy as np
from jax import lax

F32 = jnp.float32
BF16 = jnp.bfloat16
I32 = jnp.int32
LANES = 128
CHUNK = 128


def _dft_matrices(c):
    theta = np.pi * (np.arange(c)[:, None] + 0.5) * np.arange(c)[None, :] / c
    parts = np.stack([np.cos(theta), -np.sin(theta)])
    fwd = parts.reshape(2, c // 8, 8, c).transpose(1, 0, 2, 3).reshape(2 * c, c)
    return fwd.astype(np.float32), (fwd.T / c).astype(np.float32)


_FWD, _INV = _dft_matrices(CHUNK)
_NT = (((1,), (1,)), ((), ()))


def _interleave(*jobs):
    order = sorted(((i + 0.5) / n, j) for j, (_, n) in enumerate(jobs) for i in range(n))
    for _, j in order:
        next(jobs[j][0])
    for job, _ in jobs:
        for _ in job:
            pass


def _step_schedule(pairs):
    order = []
    for g in range(pairs):
        order += [("q", g), ("v", g), ("s", g - 1), ("k", g), ("o", g - 7), ("p", g - 2)]
    for op, back in zip("oospooopoo", (7, 6, 1, 2, 5, 4, 3, 1, 2, 1)):
        order.append((op, pairs - back))
    return [(op, g) for op, g in order if g >= 0]


def _kernel(
    mem0_ref, shift_ref, ssmd_ref, gate_ref, fwd_ref, inv_ref,
    x_hbm, k_hbm, v_hbm, ssm_hbm, wq_hbm, wk_hbm, wv_hbm, wo_hbm,
    out_hbm,
    x_s, k_s, v_s, ssm_s, stage_s, wqkv_s, wo_s,
    kpad_s, xf_s, kf_s, zf_s, tail_s,
    h_s, q_s, kb_s, vb_s, p_s, o_s,
    in_sems, w_sems, out_sem,
    *, seq, dm, heads, dh, nmem, seg,
):
    rows = nmem + seg
    nseg = seq // seg
    pairs = heads // 2
    pw = 2 * dh
    nchunk = seq // CHUNK
    nblk = dm // LANES
    w_hbm = (wq_hbm, wk_hbm, wv_hbm)

    ssm_copies = [
        pltpu.make_async_copy(
            ssm_hbm.at[pl.ds(i * dm // 2, dm // 2), :],
            ssm_s.at[pl.ds(i * dm // 2, dm // 2), :], in_sems.at[i])
        for i in range(2)
    ]
    k_copy = pltpu.make_async_copy(k_hbm, k_s, in_sems.at[2])
    v_copy = pltpu.make_async_copy(v_hbm, v_s, in_sems.at[3])
    x_copy = pltpu.make_async_copy(x_hbm, x_s, in_sems.at[4])

    def w_copy(m, g):
        sl = pl.ds(pl.multiple_of(g * pw, pw), pw)
        if m == 3:
            return pltpu.make_async_copy(
                wo_hbm.at[sl, :], wo_s.at[sl, :], w_sems.at[m * pairs + g])
        return pltpu.make_async_copy(
            w_hbm[m].at[sl, :], stage_s.at[m, g], w_sems.at[m * pairs + g])

    def start_qkv(g):
        for m in range(3):
            w_copy(m, g).start()

    for c in ssm_copies:
        c.start()
    for c in ssm_copies:
        c.wait()
    k_copy.start()
    v_copy.start()

    sub = lax.broadcasted_iota(I32, (8, LANES), 0)
    sign = jnp.where((sub & 1) == 0, 1.0, -1.0).astype(F32)

    def filter_spectra(j, carry):
        ch = pl.ds(pl.multiple_of(j * LANES, LANES), LANES)
        fwd = fwd_ref[...]
        prev = None
        for a in range(nchunk):
            spec = lax.dot_general(
                fwd, ssm_s[ch, a * CHUNK:(a + 1) * CHUNK], _NT,
                preferred_element_type=F32).reshape(CHUNK // 8, 2, 8, LANES)
            if prev is None:
                folded = spec
            else:
                folded = jnp.stack(
                    [spec[:, 0] - sign * prev[:, 1], spec[:, 1] + sign * prev[:, 0]],
                    axis=1)
            kf_s[j, a] = folded.reshape(2 * CHUNK, LANES)
            prev = spec
        return carry

    lax.fori_loop(0, nblk, filter_spectra, 0)
    k_copy.wait()
    v_copy.wait()
    x_copy.start()
    start_qkv(0)
    kpad_s[0:8, :] = jnp.zeros((8, LANES), F32)

    def signal_spectra(j, carry):
        ch = pl.ds(pl.multiple_of(j * LANES, LANES), LANES)
        fwd = fwd_ref[...]
        kpad_s[8:, :] = k_s[:, ch].astype(F32)
        taps = shift_ref[:, ch].astype(F32)
        for a in range(nchunk):
            t = slice(a * CHUNK, (a + 1) * CHUNK)
            acc = kpad_s[pl.ds(8 + a * CHUNK, CHUNK), :] * taps[0:1, :]
            for lag in range(1, taps.shape[0]):
                acc = acc + (
                    kpad_s[pl.ds(8 + a * CHUNK - lag, CHUNK), :] * taps[lag:lag + 1, :])
            kv = (acc * v_s[t, ch].astype(F32)).astype(BF16)
            v_s[t, ch] = kv
            xf_s[j, a] = jnp.dot(fwd, kv, preferred_element_type=F32)
        pl.when(j == nblk // 2)(functools.partial(start_qkv, 1))
        return carry

    lax.fori_loop(0, nblk, signal_spectra, 0)
    x_copy.wait()

    for s in range(nseg):
        tail_s[8 * s:8 * s + 8, :] = (
            x_s[(s + 1) * seg - 16:(s + 1) * seg, :].astype(F32)[8:])

    tail_rows = 128

    def prepare(g, carry):
        for m in range(3):
            w_copy(m, g).wait()
        pl.when(g + 2 < pairs)(lambda: start_qkv(g + 2))
        w_copy(3, g).start()

        last = [None]

        def tail_projection():
            for m in range(2):
                for n in range(pw // LANES):
                    w = stage_s[m, g, n * LANES:(n + 1) * LANES, :]
                    for r in range(0, 8 * nseg, tail_rows):
                        full = lax.dot_general(
                            tail_s[r:r + tail_rows, :], w, _NT, preferred_element_type=F32)
                        for i in range(0, tail_rows, 16):
                            word = (r + i) // 2
                            last[0] = pltpu.bitcast(full[i:i + 16].astype(BF16), F32)
                            kf_s[nblk + 3 * m + n, g, word:word + 8, :] = last[0]
                            yield

        def transpose():
            for m in range(3):
                for n in range(pw // LANES):
                    w = stage_s[m, g, n * LANES:(n + 1) * LANES, :]
                    wqkv_s[g, 0:dm // 2, m * pw + n * LANES:m * pw + (n + 1) * LANES] = (
                        pltpu.bitcast(w.T, I32))
                    wqkv_s[pairs - 1 - g, dm // 2:, 0:LANES] = pltpu.bitcast(last[0], I32)
                    yield

        def chunk_conv():
            re = pl.ds(pl.multiple_of(g * 16, 8), 8)
            im = pl.ds(pl.multiple_of(g * 16 + 8, 8), 8)
            for j in range(nblk):
                xr, xi = [], []
                for c in range(nchunk):
                    xr.append(xf_s[j, c, re, :])
                    xi.append(xf_s[j, c, im, :])
                    zr = zi = None
                    for a in range(c + 1):
                        kr = kf_s[j, c - a, re, :]
                        ki = kf_s[j, c - a, im, :]
                        tr = xr[a] * kr - xi[a] * ki
                        ti = xr[a] * ki + xi[a] * kr
                        zr = tr if zr is None else zr + tr
                        zi = ti if zi is None else zi + ti
                        yield
                    z = jnp.concatenate([zr, zi], axis=0).astype(BF16)
                    zf_s[j, c, pl.ds(pl.multiple_of(g * 8, 8), 8), :] = (
                        pltpu.bitcast(z, I32))

        _interleave(
            (tail_projection(), 2 * (pw // LANES) * nseg // 2),
            (chunk_conv(), nblk * nchunk * (nchunk + 1) // 2),
            (transpose(), 3 * (pw // LANES)),
        )
        return carry

    lax.fori_loop(0, pairs, prepare, 0)

    h_s[0:1, :] = ssmd_ref[...].astype(F32).reshape(1, dm)

    def finish_conv(j, carry):
        ch = pl.ds(pl.multiple_of(j * LANES, LANES), LANES)
        inv = inv_ref[...]
        skip = h_s[0:1, ch]
        for c in range(nchunk):
            t = slice(c * CHUNK, (c + 1) * CHUNK)
            y = jnp.dot(
                inv, pltpu.bitcast(zf_s[j, c], BF16), preferred_element_type=F32)
            y = y + v_s[t, ch].astype(F32) * skip
            kf_s[j, c, 0:CHUNK, :] = x_s[t, ch].astype(F32) * y
        return carry

    lax.fori_loop(0, nblk, finish_conv, 0)
    for g in range(pairs):
        w_copy(3, g).wait()

    scale = dh ** -0.5
    head = rows - 8
    lane = lax.broadcasted_iota(I32, (rows, LANES), 1)
    first_half = lane < (dh - LANES)
    col = lax.broadcasted_iota(I32, (rows, 2 * rows), 1)
    row = lax.broadcasted_iota(I32, (rows, 2 * rows), 0)
    head0 = col < rows
    allowed = (row < nmem) | (row >= jnp.where(head0, col, col - rows))
    zeros = jnp.zeros((rows, LANES), F32)
    gate_w = gate_ref[...].astype(F32).reshape(1, dm)
    out_s = k_s

    def block_diag(t):
        a, b, c = t[:, :LANES], t[:, LANES:2 * LANES], t[:, 2 * LANES:]
        top = jnp.concatenate([a, jnp.where(first_half, b, 0.0), zeros], axis=1)
        bot = jnp.concatenate([zeros, jnp.where(first_half, 0.0, b), c], axis=1)
        return pltpu.bitcast(jnp.concatenate([top, bot], axis=0).astype(BF16), I32)

    def project_qk(m, g, s):
        two = pl.ds(pl.multiple_of((s // 2) * 8, 8), 8)
        w = pltpu.bitcast(wqkv_s[g, 0:dm // 2, m * pw:(m + 1) * pw], BF16)
        most = jnp.dot(h_s[0:head, :], w, preferred_element_type=F32)
        words = [kf_s[nblk + 3 * m + n, g, two, :] for n in range(pw // LANES)]
        both = pltpu.bitcast(jnp.concatenate(words, axis=1), BF16).astype(F32)
        tail = jnp.where(s % 2 == 0, both[:8], both[8:])
        return jnp.concatenate([most, tail], axis=0)

    def queries(g, s):
        q_s[g] = project_qk(0, g, s)

    def keys(g, s):
        kb_s[g] = block_diag(project_qk(1, g, s))

    def vals(g):
        w = pltpu.bitcast(wqkv_s[g, 0:dm // 2, 2 * pw:], BF16)
        vb_s[g] = block_diag(jnp.dot(h_s[...], w, preferred_element_type=F32))

    def scores(g):
        s = lax.dot_general(
            q_s[g], pltpu.bitcast(kb_s[g], BF16), _NT, preferred_element_type=F32)
        s = jnp.where(allowed, s * scale, -1000000000.0)
        m0 = jnp.max(jnp.where(head0, s, -jnp.inf), axis=1, keepdims=True)
        m1 = jnp.max(jnp.where(head0, -jnp.inf, s), axis=1, keepdims=True)
        e = jnp.exp(s - jnp.where(head0, m0, m1))
        d0 = jnp.sum(jnp.where(head0, e, 0.0), axis=1, keepdims=True)
        d1 = jnp.sum(jnp.where(head0, 0.0, e), axis=1, keepdims=True)
        p_s[g] = e / jnp.where(head0, d0, d1)

    def values(g):
        o_s[:, g * pw:(g + 1) * pw] = jnp.dot(
            p_s[g], pltpu.bitcast(vb_s[g], BF16), preferred_element_type=F32)

    def out_proj(g):
        return jnp.dot(
            o_s[:, g * pw:(g + 1) * pw], wo_s[g * pw:(g + 1) * pw, :],
            preferred_element_type=F32)

    h_s[0:nmem, :] = mem0_ref[...].astype(F32)

    def segment(s, carry):
        t = pl.ds(pl.multiple_of(s * seg, seg), seg)
        xs = x_s[t, :].astype(F32)
        h_s[nmem:, :] = xs
        a = None
        for op, g in _step_schedule(pairs):
            if op == "o":
                part = out_proj(g)
                a = part if a is None else a + part
            else:
                dict(q=lambda: queries(g, s), k=lambda: keys(g, s), v=lambda: vals(g),
                     s=lambda: scores(g), p=lambda: values(g))[op]()
        h_s[0:nmem, :] = a[:nmem]
        per_chunk = CHUNK // seg
        in_chunk = pl.ds(pl.multiple_of((s % per_chunk) * seg, seg), seg)
        b = jnp.concatenate(
            [kf_s[j, s // per_chunk, in_chunk, :] for j in range(nblk)], axis=1)
        gate = jax.nn.sigmoid(jnp.sum(xs * gate_w, axis=1, keepdims=True))
        out_s[t, :] = (gate * a[nmem:] + (1.0 - gate) * b).astype(BF16)
        pltpu.make_async_copy(out_s.at[t, :], out_hbm.at[t, :], out_sem).start()
        return carry

    lax.fori_loop(0, nseg, segment, 0)
    pltpu.make_async_copy(out_s, out_hbm, out_sem).wait()


@functools.partial(jax.jit, static_argnames=("A_seg_len",))
def pallas_gated_mix__memory_aug_recurrent_mem_tr__ssm_conv_h3__prompt_kernel(
    A_x: jax.Array,
    A_mem0: jax.Array,
    A_Wq: jax.Array,
    A_Wk: jax.Array,
    A_Wv: jax.Array,
    A_Wo: jax.Array,
    A_seg_len: int,
    B_q: jax.Array,
    B_k: jax.Array,
    B_v: jax.Array,
    B_shift_k: jax.Array,
    B_ssm_k: jax.Array,
    B_ssm_D: jax.Array,
    gate_w: jax.Array,
):
    del B_q
    batch, seq, dm = A_x.shape
    _, heads, dh = A_Wq.shape
    nmem = A_mem0.shape[1]
    seg = int(A_seg_len)
    feat = heads * dh
    rows = nmem + seg
    pairs = heads // 2
    pw = 2 * dh
    nchunk = seq // CHUNK
    nblk = dm // LANES
    nseg = seq // seg
    assert pairs == CHUNK // 8 and nseg % 2 == 0 and CHUNK % seg == 0
    assert batch == 1 and dh == 192 and heads % 8 == 0 and dm % LANES == 0
    assert nmem % 8 == 0 and seg % 16 == 0 and seq % seg == 0 and 2 * rows <= LANES
    assert seq % CHUNK == 0 and B_shift_k.shape[1] <= 8

    def feature_major(w):
        return w.transpose(1, 2, 0).reshape(feat, dm)

    vmem = pl.BlockSpec(memory_space=pltpu.VMEM)
    hbm = pl.BlockSpec(memory_space=pltpu.HBM)
    out = pl.pallas_call(
        functools.partial(
            _kernel, seq=seq, dm=dm, heads=heads, dh=dh, nmem=nmem, seg=seg),
        out_shape=jax.ShapeDtypeStruct((seq, dm), BF16),
        in_specs=[vmem] * 6 + [hbm] * 8,
        out_specs=hbm,
        scratch_shapes=[
            pltpu.VMEM((seq, dm), BF16),
            pltpu.VMEM((seq, dm), BF16),
            pltpu.VMEM((seq, dm), BF16),
            pltpu.VMEM((dm, seq), BF16),
            pltpu.VMEM((3, pairs, pw, dm), BF16),
            pltpu.VMEM((pairs, dm // 2 + 8, 3 * pw), I32),
            pltpu.VMEM((feat, dm), BF16),
            pltpu.VMEM((8 + seq, LANES), F32),
            pltpu.VMEM((nblk, nchunk, 2 * CHUNK, LANES), F32),
            pltpu.VMEM((nblk + 6, nchunk, 2 * CHUNK, LANES), F32),
            pltpu.VMEM((nblk, nchunk, CHUNK, LANES), I32),
            pltpu.VMEM((8 * nseg, dm), F32),
            pltpu.VMEM((rows, dm), F32),
            pltpu.VMEM((pairs, rows, pw), F32),
            pltpu.VMEM((pairs, rows, pw), I32),
            pltpu.VMEM((pairs, rows, pw), I32),
            pltpu.VMEM((pairs, rows, 2 * rows), F32),
            pltpu.VMEM((rows, feat), F32),
            pltpu.SemaphoreType.DMA((5,)),
            pltpu.SemaphoreType.DMA((4 * pairs,)),
            pltpu.SemaphoreType.DMA,
        ],
        compiler_params=pltpu.CompilerParams(vmem_limit_bytes=112 * 1024 * 1024),
        name="gated_mix_mem_h3",
    )(
        A_mem0.reshape(nmem, dm),
        B_shift_k.T,
        B_ssm_D,
        gate_w,
        jnp.asarray(_FWD, BF16),
        jnp.asarray(_INV, BF16),
        A_x.reshape(seq, dm),
        B_k.reshape(seq, dm),
        B_v.reshape(seq, dm),
        B_ssm_k,
        feature_major(A_Wq),
        feature_major(A_Wk),
        feature_major(A_Wv),
        A_Wo.reshape(feat, dm),
    )
    return out.reshape(batch, seq, dm)
```

```python
import functools

import jax
import jax.experimental.pallas as pl
import jax.experimental.pallas.tpu as pltpu
import jax.numpy as jnp
import numpy as np
from jax import lax

F32 = jnp.float32
BF16 = jnp.bfloat16
I32 = jnp.int32
LANES = 128
CHUNK = 128


def _dft_matrices(c):
    theta = np.pi * (np.arange(c)[:, None] + 0.5) * np.arange(c)[None, :] / c
    parts = np.stack([np.cos(theta), -np.sin(theta)])
    fwd = parts.reshape(2, c // 8, 8, c).transpose(1, 0, 2, 3).reshape(2 * c, c)
    return fwd.astype(np.float32), (fwd.T / c).astype(np.float32)


_FWD, _INV = _dft_matrices(CHUNK)
_NT = (((1,), (1,)), ((), ()))


def _interleave(*jobs):
    order = sorted(((i + 0.5) / n, j) for j, (_, n) in enumerate(jobs) for i in range(n))
    for _, j in order:
        next(jobs[j][0])
    for job, _ in jobs:
        for _ in job:
            pass


def _step_schedule(pairs):
    order = []
    for g in range(pairs):
        order += [("q", g), ("v", g), ("s", g - 1), ("k", g), ("o", g - 7), ("p", g - 2)]
    for op, back in zip("oospooopoo", (7, 6, 1, 2, 5, 4, 3, 1, 2, 1)):
        order.append((op, pairs - back))
    return [(op, g) for op, g in order if g >= 0]


def _kernel(
    mem0_ref, shift_ref, ssmd_ref, gate_ref, fwd_ref, inv_ref,
    x_hbm, xseg_hbm, k_hbm, v_hbm, ssm_hbm, wq_hbm, wk_hbm, wv_hbm, wo_hbm,
    out_hbm,
    x_s, xtail_s, k_s, v_s, ssm_s, stage_s, wqkv_s, wo_s,
    kpad_s, xf_s, kf_s, zf_s, tail_s,
    h_s, q_s, kb_s, vb_s, p_s, o_s,
    in_sems, w_sems, out_sem,
    *, seq, dm, heads, dh, nmem, seg,
):
    rows = nmem + seg
    nseg = seq // seg
    pairs = heads // 2
    pw = 2 * dh
    nchunk = seq // CHUNK
    nblk = dm // LANES
    w_hbm = (wq_hbm, wk_hbm, wv_hbm)

    def block_copies(j):
        ch = pl.ds(pl.multiple_of(j * LANES, LANES), LANES)
        return [
            pltpu.make_async_copy(src, dst, in_sems.at[3 * j + i])
            for i, (src, dst) in enumerate((
                (ssm_hbm.at[ch, :], ssm_s.at[ch, :]),
                (k_hbm.at[:, ch], k_s.at[:, ch]),
                (v_hbm.at[:, ch], v_s.at[:, ch])))
        ]

    x_copy = pltpu.make_async_copy(x_hbm, x_s, in_sems.at[3 * nblk])
    xtail_copy = pltpu.make_async_copy(
        xseg_hbm.at[:, pl.ds(seg - 8, 8), :], xtail_s, in_sems.at[3 * nblk + 1])

    def w_copy(m, g):
        sl = pl.ds(pl.multiple_of(g * pw, pw), pw)
        if m == 3:
            return pltpu.make_async_copy(
                wo_hbm.at[sl, :], wo_s.at[sl, :], w_sems.at[m * pairs + g])
        return pltpu.make_async_copy(
            w_hbm[m].at[sl, :], stage_s.at[m, g], w_sems.at[m * pairs + g])

    def start_qkv(g):
        for m in range(3):
            w_copy(m, g).start()

    def start_block(j):
        for c in block_copies(j):
            c.start()

    ahead = 2
    start_block(0)
    start_block(1)
    xtail_copy.start()
    kpad_s[0:8, :] = jnp.zeros((8, LANES), F32)
    sub = lax.broadcasted_iota(I32, (8, LANES), 0)
    sign = jnp.where((sub & 1) == 0, 1.0, -1.0).astype(F32)

    def spectra(j, carry):
        for c in block_copies(j):
            c.wait()
        pl.when(j + 2 < nblk)(lambda: start_block(j + 2))
        pl.when(j + ahead >= nblk)(lambda: start_qkv(j + ahead - nblk))

        ch = pl.ds(pl.multiple_of(j * LANES, LANES), LANES)
        fwd = fwd_ref[...]
        kpad_s[8:, :] = k_s[:, ch].astype(F32)
        taps = shift_ref[:, ch].astype(F32)
        prev = None
        for a in range(nchunk):
            t = slice(a * CHUNK, (a + 1) * CHUNK)
            spec = lax.dot_general(
                fwd, ssm_s[ch, t], _NT, preferred_element_type=F32
            ).reshape(CHUNK // 8, 2, 8, LANES)
            if prev is None:
                folded = spec
            else:
                folded = jnp.stack(
                    [spec[:, 0] - sign * prev[:, 1], spec[:, 1] + sign * prev[:, 0]],
                    axis=1)
            kf_s[j, a, 0:2 * CHUNK, :] = folded.reshape(2 * CHUNK, LANES)
            prev = spec
            acc = kpad_s[pl.ds(8 + a * CHUNK, CHUNK), :] * taps[0:1, :]
            for lag in range(1, taps.shape[0]):
                acc = acc + (
                    kpad_s[pl.ds(8 + a * CHUNK - lag, CHUNK), :] * taps[lag:lag + 1, :])
            kv = (acc * v_s[t, ch].astype(F32)).astype(BF16)
            v_s[t, ch] = kv
            xf_s[j, a, 0:2 * CHUNK, :] = jnp.dot(fwd, kv, preferred_element_type=F32)
        return carry

    lax.fori_loop(0, nblk, spectra, 0)
    xtail_copy.wait()

    for s in range(nseg):
        tail_s[8 * s:8 * s + 8, :] = xtail_s[s].astype(F32)

    tail_rows = 128

    def prepare(g, carry):
        for m in range(3):
            w_copy(m, g).wait()
        pl.when(g + ahead < pairs)(lambda: start_qkv(g + ahead))
        w_copy(3, g).start()
        pl.when(g + ahead + 1 == pairs)(x_copy.start)

        last = [None]

        def tail_projection():
            for m in range(2):
                for n in range(pw // LANES):
                    w = stage_s[m, g, n * LANES:(n + 1) * LANES, :]
                    for r in range(0, 8 * nseg, tail_rows):
                        full = lax.dot_general(
                            tail_s[r:r + tail_rows, :], w, _NT, preferred_element_type=F32)
                        for i in range(0, tail_rows, 16):
                            word = (r + i) // 2
                            last[0] = pltpu.bitcast(full[i:i + 16].astype(BF16), F32)
                            kf_s[nblk + 3 * m + n, g, word:word + 8, :] = last[0]
                            yield

        def transpose():
            for m in range(3):
                for n in range(pw // LANES):
                    w = stage_s[m, g, n * LANES:(n + 1) * LANES, :]
                    wqkv_s[g, 0:dm // 2, m * pw + n * LANES:m * pw + (n + 1) * LANES] = (
                        pltpu.bitcast(w.T, I32))
                    wqkv_s[pairs - 1 - g, dm // 2:, 0:LANES] = pltpu.bitcast(last[0], I32)
                    yield

        def chunk_conv():
            re = pl.ds(pl.multiple_of(g * 16, 8), 8)
            im = pl.ds(pl.multiple_of(g * 16 + 8, 8), 8)
            for j in range(nblk):
                xr, xi = [], []
                for c in range(nchunk):
                    xr.append(xf_s[j, c, re, :])
                    xi.append(xf_s[j, c, im, :])
                    zr = zi = None
                    for a in range(c + 1):
                        kr = kf_s[j, c - a, re, :]
                        ki = kf_s[j, c - a, im, :]
                        tr = xr[a] * kr - xi[a] * ki
                        ti = xr[a] * ki + xi[a] * kr
                        zr = tr if zr is None else zr + tr
                        zi = ti if zi is None else zi + ti
                        yield
                    z = jnp.concatenate([zr, zi], axis=0).astype(BF16)
                    zf_s[j, c, pl.ds(pl.multiple_of(g * 8, 8), 8), :] = (
                        pltpu.bitcast(z, I32))

        _interleave(
            (tail_projection(), 2 * (pw // LANES) * nseg // 2),
            (chunk_conv(), nblk * nchunk * (nchunk + 1) // 2),
            (transpose(), 3 * (pw // LANES)),
        )
        return carry

    lax.fori_loop(0, pairs, prepare, 0)

    x_copy.wait()
    h_s[0:1, :] = ssmd_ref[...].astype(F32).reshape(1, dm)

    def finish_conv(j, carry):
        ch = pl.ds(pl.multiple_of(j * LANES, LANES), LANES)
        inv = inv_ref[...]
        skip = h_s[0:1, ch]
        for c in range(nchunk):
            t = slice(c * CHUNK, (c + 1) * CHUNK)
            y = jnp.dot(
                inv, pltpu.bitcast(zf_s[j, c], BF16), preferred_element_type=F32)
            y = y + v_s[t, ch].astype(F32) * skip
            kf_s[j, c, 0:CHUNK, :] = x_s[t, ch].astype(F32) * y
        return carry

    lax.fori_loop(0, nblk, finish_conv, 0)
    for g in range(pairs):
        w_copy(3, g).wait()

    scale = dh ** -0.5
    head = rows - 8
    lane = lax.broadcasted_iota(I32, (rows, LANES), 1)
    first_half = lane < (dh - LANES)
    col = lax.broadcasted_iota(I32, (rows, 2 * rows), 1)
    row = lax.broadcasted_iota(I32, (rows, 2 * rows), 0)
    head0 = col < rows
    allowed = (row < nmem) | (row >= jnp.where(head0, col, col - rows))
    zeros = jnp.zeros((rows, LANES), F32)
    gate_w = gate_ref[...].astype(F32).reshape(1, dm)
    out_s = k_s

    def block_diag(t):
        a, b, c = t[:, :LANES], t[:, LANES:2 * LANES], t[:, 2 * LANES:]
        top = jnp.concatenate([a, jnp.where(first_half, b, 0.0), zeros], axis=1)
        bot = jnp.concatenate([zeros, jnp.where(first_half, 0.0, b), c], axis=1)
        return pltpu.bitcast(jnp.concatenate([top, bot], axis=0).astype(BF16), I32)

    def project_qk(m, g, s):
        two = pl.ds(pl.multiple_of((s // 2) * 8, 8), 8)
        w = pltpu.bitcast(wqkv_s[g, 0:dm // 2, m * pw:(m + 1) * pw], BF16)
        most = jnp.dot(h_s[0:head, :], w, preferred_element_type=F32)
        words = [kf_s[nblk + 3 * m + n, g, two, :] for n in range(pw // LANES)]
        both = pltpu.bitcast(jnp.concatenate(words, axis=1), BF16).astype(F32)
        tail = jnp.where(s % 2 == 0, both[:8], both[8:])
        return jnp.concatenate([most, tail], axis=0)

    def queries(g, s):
        q_s[g] = project_qk(0, g, s)

    def keys(g, s):
        kb_s[g] = block_diag(project_qk(1, g, s))

    def vals(g):
        w = pltpu.bitcast(wqkv_s[g, 0:dm // 2, 2 * pw:], BF16)
        vb_s[g] = block_diag(jnp.dot(h_s[...], w, preferred_element_type=F32))

    def scores(g):
        s = lax.dot_general(
            q_s[g], pltpu.bitcast(kb_s[g], BF16), _NT, preferred_element_type=F32)
        s = jnp.where(allowed, s * scale, -1000000000.0)
        m0 = jnp.max(jnp.where(head0, s, -jnp.inf), axis=1, keepdims=True)
        m1 = jnp.max(jnp.where(head0, -jnp.inf, s), axis=1, keepdims=True)
        e = jnp.exp(s - jnp.where(head0, m0, m1))
        d0 = jnp.sum(jnp.where(head0, e, 0.0), axis=1, keepdims=True)
        d1 = jnp.sum(jnp.where(head0, 0.0, e), axis=1, keepdims=True)
        p_s[g] = e / jnp.where(head0, d0, d1)

    def values(g):
        o_s[:, g * pw:(g + 1) * pw] = jnp.dot(
            p_s[g], pltpu.bitcast(vb_s[g], BF16), preferred_element_type=F32)

    def out_proj(g):
        return jnp.dot(
            o_s[:, g * pw:(g + 1) * pw], wo_s[g * pw:(g + 1) * pw, :],
            preferred_element_type=F32)

    h_s[0:nmem, :] = mem0_ref[...].astype(F32)

    def segment(s, carry):
        t = pl.ds(pl.multiple_of(s * seg, seg), seg)
        xs = x_s[t, :].astype(F32)
        h_s[nmem:, :] = xs
        a = None
        for op, g in _step_schedule(pairs):
            if op == "o":
                part = out_proj(g)
                a = part if a is None else a + part
            else:
                dict(q=lambda: queries(g, s), k=lambda: keys(g, s), v=lambda: vals(g),
                     s=lambda: scores(g), p=lambda: values(g))[op]()
        h_s[0:nmem, :] = a[:nmem]
        per_chunk = CHUNK // seg
        in_chunk = pl.ds(pl.multiple_of((s % per_chunk) * seg, seg), seg)
        b = jnp.concatenate(
            [kf_s[j, s // per_chunk, in_chunk, :] for j in range(nblk)], axis=1)
        gate = jax.nn.sigmoid(jnp.sum(xs * gate_w, axis=1, keepdims=True))
        out_s[t, :] = (gate * a[nmem:] + (1.0 - gate) * b).astype(BF16)
        pltpu.make_async_copy(out_s.at[t, :], out_hbm.at[t, :], out_sem).start()
        return carry

    lax.fori_loop(0, nseg, segment, 0)
    pltpu.make_async_copy(out_s, out_hbm, out_sem).wait()


@functools.partial(jax.jit, static_argnames=("A_seg_len",))
def pallas_gated_mix__memory_aug_recurrent_mem_tr__ssm_conv_h3__prompt_kernel(
    A_x: jax.Array,
    A_mem0: jax.Array,
    A_Wq: jax.Array,
    A_Wk: jax.Array,
    A_Wv: jax.Array,
    A_Wo: jax.Array,
    A_seg_len: int,
    B_q: jax.Array,
    B_k: jax.Array,
    B_v: jax.Array,
    B_shift_k: jax.Array,
    B_ssm_k: jax.Array,
    B_ssm_D: jax.Array,
    gate_w: jax.Array,
):
    del B_q
    batch, seq, dm = A_x.shape
    _, heads, dh = A_Wq.shape
    nmem = A_mem0.shape[1]
    seg = int(A_seg_len)
    feat = heads * dh
    rows = nmem + seg
    pairs = heads // 2
    pw = 2 * dh
    nchunk = seq // CHUNK
    nblk = dm // LANES
    nseg = seq // seg
    assert pairs == CHUNK // 8 and nseg % 2 == 0 and CHUNK % seg == 0
    assert batch == 1 and dh == 192 and heads % 8 == 0 and dm % LANES == 0
    assert nmem % 8 == 0 and seg % 16 == 0 and seq % seg == 0 and 2 * rows <= LANES
    assert seq % CHUNK == 0 and B_shift_k.shape[1] <= 8

    def feature_major(w):
        return w.transpose(1, 2, 0).reshape(feat, dm)

    vmem = pl.BlockSpec(memory_space=pltpu.VMEM)
    hbm = pl.BlockSpec(memory_space=pltpu.HBM)
    out = pl.pallas_call(
        functools.partial(
            _kernel, seq=seq, dm=dm, heads=heads, dh=dh, nmem=nmem, seg=seg),
        out_shape=jax.ShapeDtypeStruct((seq, dm), BF16),
        in_specs=[vmem] * 6 + [hbm] * 9,
        out_specs=hbm,
        scratch_shapes=[
            pltpu.VMEM((seq, dm), BF16),
            pltpu.VMEM((nseg, 8, dm), BF16),
            pltpu.VMEM((seq, dm), BF16),
            pltpu.VMEM((seq, dm), BF16),
            pltpu.VMEM((dm, seq), BF16),
            pltpu.VMEM((3, pairs, pw, dm), BF16),
            pltpu.VMEM((pairs, dm // 2 + 8, 3 * pw), I32),
            pltpu.VMEM((feat, dm), BF16),
            pltpu.VMEM((8 + seq, LANES), F32),
            pltpu.VMEM((nblk, nchunk, 2 * CHUNK + 8, LANES), F32),
            pltpu.VMEM((nblk + 6, nchunk, 2 * CHUNK + 24, LANES), F32),
            pltpu.VMEM((nblk, nchunk, CHUNK, LANES), I32),
            pltpu.VMEM((8 * nseg, dm), F32),
            pltpu.VMEM((rows, dm), F32),
            pltpu.VMEM((pairs, rows, pw), F32),
            pltpu.VMEM((pairs, rows, pw), I32),
            pltpu.VMEM((pairs, rows, pw), I32),
            pltpu.VMEM((pairs, rows, 2 * rows), F32),
            pltpu.VMEM((rows, feat), F32),
            pltpu.SemaphoreType.DMA((3 * nblk + 2,)),
            pltpu.SemaphoreType.DMA((4 * pairs,)),
            pltpu.SemaphoreType.DMA,
        ],
        compiler_params=pltpu.CompilerParams(vmem_limit_bytes=112 * 1024 * 1024),
        name="gated_mix_mem_h3",
    )(
        A_mem0.reshape(nmem, dm),
        B_shift_k.T,
        B_ssm_D,
        gate_w,
        jnp.asarray(_FWD, BF16),
        jnp.asarray(_INV, BF16),
        A_x.reshape(seq, dm),
        A_x.reshape(nseg, seg, dm),
        B_k.reshape(seq, dm),
        B_v.reshape(seq, dm),
        B_ssm_k,
        feature_major(A_Wq),
        feature_major(A_Wk),
        feature_major(A_Wv),
        A_Wo.reshape(feat, dm),
    )
    return out.reshape(batch, seq, dm)
```

```python
import functools

import jax
import jax.experimental.pallas as pl
import jax.experimental.pallas.tpu as pltpu
import jax.numpy as jnp
import numpy as np
from jax import lax

F32 = jnp.float32
BF16 = jnp.bfloat16
I32 = jnp.int32
LANES = 128
CHUNK = 128


def _dft_matrices(c):
    theta = np.pi * (np.arange(c)[:, None] + 0.5) * np.arange(c)[None, :] / c
    parts = np.stack([np.cos(theta), -np.sin(theta)])
    fwd = parts.reshape(2, c // 8, 8, c).transpose(1, 0, 2, 3).reshape(2 * c, c)
    return fwd.astype(np.float32), (fwd.T / c).astype(np.float32)


_FWD, _INV = _dft_matrices(CHUNK)
_NT = (((1,), (1,)), ((), ()))


def _interleave(*jobs):
    order = sorted(((i + 0.5) / n, j) for j, (_, n) in enumerate(jobs) for i in range(n))
    for _, j in order:
        next(jobs[j][0])
    for job, _ in jobs:
        for _ in job:
            pass


def _step_schedule(pairs):
    body = "q0 v0 s1 k0 o7 p2"
    drain = "o7 o6 s1 p2 o5 o4 o3 p1 o2 o1 c0"
    order = [(t[0], g - int(t[1:])) for g in range(pairs) for t in body.split()]
    order += [(t[0], pairs - int(t[1:])) for t in drain.split()]
    return [(op, g) for op, g in order if g >= 0]


def _kernel(
    mem0_ref, shift_ref, ssmd_ref, gate_ref, fwd_ref, inv_ref,
    x_hbm, xseg_hbm, k_hbm, v_hbm, ssm_hbm, wq_hbm, wk_hbm, wv_hbm, wo_hbm,
    out_hbm,
    x_s, xtail_s, k_s, v_s, ssm_s, stage_s, wqkv_s, wo_s,
    kpad_s, xf_s, kf_s, zf_s, tail_s,
    h_s, q_s, kb_s, vb_s, p_s, o_s,
    in_sems, w_sems, out_sem,
    *, seq, dm, heads, dh, nmem, seg,
):
    rows = nmem + seg
    nseg = seq // seg
    pairs = heads // 2
    pw = 2 * dh
    nchunk = seq // CHUNK
    nblk = dm // LANES
    w_hbm = (wq_hbm, wk_hbm, wv_hbm)

    def block_copies(j):
        ch = pl.ds(pl.multiple_of(j * LANES, LANES), LANES)
        return [
            pltpu.make_async_copy(src, dst, in_sems.at[3 * j + i])
            for i, (src, dst) in enumerate((
                (ssm_hbm.at[ch, :], ssm_s.at[ch, :]),
                (k_hbm.at[:, ch], k_s.at[:, ch]),
                (v_hbm.at[:, ch], v_s.at[:, ch])))
        ]

    x_copy = pltpu.make_async_copy(x_hbm, x_s, in_sems.at[3 * nblk])
    xtail_copy = pltpu.make_async_copy(
        xseg_hbm.at[:, pl.ds(seg - 8, 8), :], xtail_s, in_sems.at[3 * nblk + 1])

    def w_copy(m, g):
        sl = pl.ds(pl.multiple_of(g * pw, pw), pw)
        if m == 3:
            return pltpu.make_async_copy(
                wo_hbm.at[sl, :], wo_s.at[sl, :], w_sems.at[m * pairs + g])
        return pltpu.make_async_copy(
            w_hbm[m].at[sl, :], stage_s.at[m, g], w_sems.at[m * pairs + g])

    def start_qkv(g):
        for m in range(3):
            w_copy(m, g).start()

    def start_block(j):
        for c in block_copies(j):
            c.start()

    ahead = 2
    start_block(0)
    start_block(1)
    xtail_copy.start()
    kpad_s[0:8, :] = jnp.zeros((8, LANES), F32)
    sub = lax.broadcasted_iota(I32, (8, LANES), 0)
    sign = jnp.where((sub & 1) == 0, 1.0, -1.0).astype(F32)

    def spectra(j, carry):
        for c in block_copies(j):
            c.wait()
        pl.when(j + 2 < nblk)(lambda: start_block(j + 2))
        pl.when(j + ahead >= nblk)(lambda: start_qkv(j + ahead - nblk))

        ch = pl.ds(pl.multiple_of(j * LANES, LANES), LANES)
        fwd = fwd_ref[...]
        kpad_s[8:, :] = k_s[:, ch].astype(F32)
        taps = shift_ref[:, ch].astype(F32)
        prev = None
        for a in range(nchunk):
            t = slice(a * CHUNK, (a + 1) * CHUNK)
            spec = lax.dot_general(
                fwd, ssm_s[ch, t], _NT, preferred_element_type=F32
            ).reshape(CHUNK // 8, 2, 8, LANES)
            if prev is None:
                folded = spec
            else:
                folded = jnp.stack(
                    [spec[:, 0] - sign * prev[:, 1], spec[:, 1] + sign * prev[:, 0]],
                    axis=1)
            kf_s[j, a, 0:2 * CHUNK, :] = folded.reshape(2 * CHUNK, LANES)
            prev = spec
            acc = kpad_s[pl.ds(8 + a * CHUNK, CHUNK), :] * taps[0:1, :]
            for lag in range(1, taps.shape[0]):
                acc = acc + (
                    kpad_s[pl.ds(8 + a * CHUNK - lag, CHUNK), :] * taps[lag:lag + 1, :])
            kv = (acc * v_s[t, ch].astype(F32)).astype(BF16)
            v_s[t, ch] = kv
            xf_s[j, a, 0:2 * CHUNK, :] = jnp.dot(fwd, kv, preferred_element_type=F32)
        return carry

    lax.fori_loop(0, nblk, spectra, 0)
    xtail_copy.wait()

    for s in range(nseg):
        tail_s[8 * s:8 * s + 8, :] = xtail_s[s].astype(F32)

    tail_rows = 128

    def prepare(g, carry):
        for m in range(3):
            w_copy(m, g).wait()
        pl.when(g + ahead < pairs)(lambda: start_qkv(g + ahead))
        w_copy(3, g).start()
        pl.when(g + ahead + 1 == pairs)(x_copy.start)

        last = [None]

        def tail_projection():
            for m in range(2):
                for n in range(pw // LANES):
                    w = stage_s[m, g, n * LANES:(n + 1) * LANES, :]
                    for r in range(0, 8 * nseg, tail_rows):
                        full = lax.dot_general(
                            tail_s[r:r + tail_rows, :], w, _NT, preferred_element_type=F32)
                        for i in range(0, tail_rows, 16):
                            word = (r + i) // 2
                            last[0] = pltpu.bitcast(full[i:i + 16].astype(BF16), F32)
                            kf_s[nblk + 3 * m + n, g, word:word + 8, :] = last[0]
                            yield

        def transpose():
            for m in range(3):
                for n in range(pw // LANES):
                    w = stage_s[m, g, n * LANES:(n + 1) * LANES, :]
                    wqkv_s[g, 0:dm // 2, m * pw + n * LANES:m * pw + (n + 1) * LANES] = (
                        pltpu.bitcast(w.T, I32))
                    wqkv_s[pairs - 1 - g, dm // 2:, 0:LANES] = pltpu.bitcast(last[0], I32)
                    yield

        def chunk_conv():
            re = pl.ds(pl.multiple_of(g * 16, 8), 8)
            im = pl.ds(pl.multiple_of(g * 16 + 8, 8), 8)
            for j in range(nblk):
                xr, xi = [], []
                for c in range(nchunk):
                    xr.append(xf_s[j, c, re, :])
                    xi.append(xf_s[j, c, im, :])
                    zr = zi = None
                    for a in range(c + 1):
                        kr = kf_s[j, c - a, re, :]
                        ki = kf_s[j, c - a, im, :]
                        tr = xr[a] * kr - xi[a] * ki
                        ti = xr[a] * ki + xi[a] * kr
                        zr = tr if zr is None else zr + tr
                        zi = ti if zi is None else zi + ti
                        yield
                    z = jnp.concatenate([zr, zi], axis=0).astype(BF16)
                    zf_s[j, c, pl.ds(pl.multiple_of(g * 8, 8), 8), :] = (
                        pltpu.bitcast(z, I32))

        _interleave(
            (tail_projection(), 2 * (pw // LANES) * nseg // 2),
            (chunk_conv(), nblk * nchunk * (nchunk + 1) // 2),
            (transpose(), 3 * (pw // LANES)),
        )
        return carry

    lax.fori_loop(0, pairs, prepare, 0)

    x_copy.wait()
    for g in range(pairs):
        w_copy(3, g).wait()

    scale = dh ** -0.5
    head = rows - 8
    lane = lax.broadcasted_iota(I32, (rows, LANES), 1)
    first_half = lane < (dh - LANES)
    col = lax.broadcasted_iota(I32, (rows, 2 * rows), 1)
    row = lax.broadcasted_iota(I32, (rows, 2 * rows), 0)
    head0 = col < rows
    allowed = (row < nmem) | (row >= jnp.where(head0, col, col - rows))
    zeros = jnp.zeros((rows, LANES), F32)
    gate_w = gate_ref[...].astype(F32).reshape(1, dm)
    skip = ssmd_ref[...].astype(F32).reshape(1, dm)
    out_s = k_s

    def block_diag(t):
        a, b, c = t[:, :LANES], t[:, LANES:2 * LANES], t[:, 2 * LANES:]
        top = jnp.concatenate([a, jnp.where(first_half, b, 0.0), zeros], axis=1)
        bot = jnp.concatenate([zeros, jnp.where(first_half, 0.0, b), c], axis=1)
        return pltpu.bitcast(jnp.concatenate([top, bot], axis=0).astype(BF16), I32)

    def project_qk(m, g, s):
        two = pl.ds(pl.multiple_of((s // 2) * 8, 8), 8)
        w = pltpu.bitcast(wqkv_s[g, 0:dm // 2, m * pw:(m + 1) * pw], BF16)
        most = jnp.dot(h_s[0:head, :], w, preferred_element_type=F32)
        words = [kf_s[nblk + 3 * m + n, g, two, :] for n in range(pw // LANES)]
        both = pltpu.bitcast(jnp.concatenate(words, axis=1), BF16).astype(F32)
        tail = jnp.where(s % 2 == 0, both[:8], both[8:])
        return jnp.concatenate([most, tail], axis=0)

    def queries(g, s):
        q_s[g] = project_qk(0, g, s)

    def keys(g, s):
        kb_s[g] = block_diag(project_qk(1, g, s))

    def vals(g, s):
        w = pltpu.bitcast(wqkv_s[g, 0:dm // 2, 2 * pw:], BF16)
        vb_s[g] = block_diag(jnp.dot(h_s[...], w, preferred_element_type=F32))

    def scores(g, s):
        sc = lax.dot_general(
            q_s[g], pltpu.bitcast(kb_s[g], BF16), _NT, preferred_element_type=F32)
        sc = jnp.where(allowed, sc * scale, -1000000000.0)
        m0 = jnp.max(jnp.where(head0, sc, -jnp.inf), axis=1, keepdims=True)
        m1 = jnp.max(jnp.where(head0, -jnp.inf, sc), axis=1, keepdims=True)
        e = jnp.exp(sc - jnp.where(head0, m0, m1))
        d0 = jnp.sum(jnp.where(head0, e, 0.0), axis=1, keepdims=True)
        d1 = jnp.sum(jnp.where(head0, 0.0, e), axis=1, keepdims=True)
        p_s[g] = e / jnp.where(head0, d0, d1)

    def weighted(g, s):
        o_s[:, g * pw:(g + 1) * pw] = jnp.dot(
            p_s[g], pltpu.bitcast(vb_s[g], BF16), preferred_element_type=F32)

    def out_proj(g):
        return jnp.dot(
            o_s[:, g * pw:(g + 1) * pw], wo_s[g * pw:(g + 1) * pw, :],
            preferred_element_type=F32)

    def long_conv(s, xs):
        per_chunk = CHUNK // seg
        inv = inv_ref[pl.ds(pl.multiple_of((s % per_chunk) * seg, seg), seg), :]
        spec = jnp.concatenate(
            [zf_s[j, s // per_chunk] for j in range(nblk)], axis=1)
        y = jnp.dot(inv, pltpu.bitcast(spec, BF16), preferred_element_type=F32)
        kv = v_s[pl.ds(pl.multiple_of(s * seg, seg), seg), :].astype(F32)
        return xs * (y + kv * skip)

    h_s[0:nmem, :] = mem0_ref[...].astype(F32)

    def segment(s, carry):
        t = pl.ds(pl.multiple_of(s * seg, seg), seg)
        xs = x_s[t, :].astype(F32)
        h_s[nmem:, :] = xs
        a = b = None
        for op, g in _step_schedule(pairs):
            if op == "o":
                a = out_proj(g) if a is None else a + out_proj(g)
            elif op == "c":
                b = long_conv(s, xs)
            else:
                dict(q=queries, k=keys, v=vals, s=scores, p=weighted)[op](g, s)
        h_s[0:nmem, :] = a[:nmem]
        gate = jax.nn.sigmoid(jnp.sum(xs * gate_w, axis=1, keepdims=True))
        out_s[t, :] = (gate * a[nmem:] + (1.0 - gate) * b).astype(BF16)
        pltpu.make_async_copy(out_s.at[t, :], out_hbm.at[t, :], out_sem).start()
        return carry

    lax.fori_loop(0, nseg, segment, 0, unroll=2)
    pltpu.make_async_copy(out_s, out_hbm, out_sem).wait()


@functools.partial(jax.jit, static_argnames=("A_seg_len",))
def pallas_gated_mix__memory_aug_recurrent_mem_tr__ssm_conv_h3__prompt_kernel(
    A_x: jax.Array,
    A_mem0: jax.Array,
    A_Wq: jax.Array,
    A_Wk: jax.Array,
    A_Wv: jax.Array,
    A_Wo: jax.Array,
    A_seg_len: int,
    B_q: jax.Array,
    B_k: jax.Array,
    B_v: jax.Array,
    B_shift_k: jax.Array,
    B_ssm_k: jax.Array,
    B_ssm_D: jax.Array,
    gate_w: jax.Array,
):
    del B_q
    batch, seq, dm = A_x.shape
    _, heads, dh = A_Wq.shape
    nmem = A_mem0.shape[1]
    seg = int(A_seg_len)
    feat = heads * dh
    rows = nmem + seg
    pairs = heads // 2
    pw = 2 * dh
    nchunk = seq // CHUNK
    nblk = dm // LANES
    nseg = seq // seg
    assert pairs == CHUNK // 8 and nseg % 2 == 0 and CHUNK % seg == 0
    assert batch == 1 and dh == 192 and heads % 8 == 0 and dm % LANES == 0
    assert nmem % 8 == 0 and seg % 16 == 0 and seq % seg == 0 and 2 * rows <= LANES
    assert seq % CHUNK == 0 and B_shift_k.shape[1] <= 8

    def feature_major(w):
        return w.transpose(1, 2, 0).reshape(feat, dm)

    vmem = pl.BlockSpec(memory_space=pltpu.VMEM)
    hbm = pl.BlockSpec(memory_space=pltpu.HBM)
    out = pl.pallas_call(
        functools.partial(
            _kernel, seq=seq, dm=dm, heads=heads, dh=dh, nmem=nmem, seg=seg),
        out_shape=jax.ShapeDtypeStruct((seq, dm), BF16),
        in_specs=[vmem] * 6 + [hbm] * 9,
        out_specs=hbm,
        scratch_shapes=[
            pltpu.VMEM((seq, dm), BF16),
            pltpu.VMEM((nseg, 8, dm), BF16),
            pltpu.VMEM((seq, dm), BF16),
            pltpu.VMEM((seq, dm), BF16),
            pltpu.VMEM((dm, seq), BF16),
            pltpu.VMEM((3, pairs, pw, dm), BF16),
            pltpu.VMEM((pairs, dm // 2 + 8, 3 * pw), I32),
            pltpu.VMEM((feat, dm), BF16),
            pltpu.VMEM((8 + seq, LANES), F32),
            pltpu.VMEM((nblk, nchunk, 2 * CHUNK + 8, LANES), F32),
            pltpu.VMEM((nblk + 6, nchunk, 2 * CHUNK + 24, LANES), F32),
            pltpu.VMEM((nblk, nchunk, CHUNK, LANES), I32),
            pltpu.VMEM((8 * nseg, dm), F32),
            pltpu.VMEM((rows, dm), F32),
            pltpu.VMEM((pairs, rows, pw), F32),
            pltpu.VMEM((pairs, rows, pw), I32),
            pltpu.VMEM((pairs, rows, pw), I32),
            pltpu.VMEM((pairs, rows, 2 * rows), F32),
            pltpu.VMEM((rows, feat), F32),
            pltpu.SemaphoreType.DMA((3 * nblk + 2,)),
            pltpu.SemaphoreType.DMA((4 * pairs,)),
            pltpu.SemaphoreType.DMA,
        ],
        compiler_params=pltpu.CompilerParams(vmem_limit_bytes=112 * 1024 * 1024),
        name="gated_mix_mem_h3",
    )(
        A_mem0.reshape(nmem, dm),
        B_shift_k.T,
        B_ssm_D,
        gate_w,
        jnp.asarray(_FWD, BF16),
        jnp.asarray(_INV, BF16),
        A_x.reshape(seq, dm),
        A_x.reshape(nseg, seg, dm),
        B_k.reshape(seq, dm),
        B_v.reshape(seq, dm),
        B_ssm_k,
        feature_major(A_Wq),
        feature_major(A_Wk),
        feature_major(A_Wv),
        A_Wo.reshape(feat, dm),
    )
    return out.reshape(batch, seq, dm)
```

```python
import functools

import jax
import jax.experimental.pallas as pl
import jax.experimental.pallas.tpu as pltpu
import jax.numpy as jnp
import numpy as np
from jax import lax

F32 = jnp.float32
BF16 = jnp.bfloat16
I32 = jnp.int32
LANES = 128
CHUNK = 128


def _dft_matrices(c):
    theta = np.pi * (np.arange(c)[:, None] + 0.5) * np.arange(c)[None, :] / c
    parts = np.stack([np.cos(theta), -np.sin(theta)])
    fwd = parts.reshape(2, c // 8, 8, c).transpose(1, 0, 2, 3).reshape(2 * c, c)
    return fwd.astype(BF16), (fwd.T / c).astype(BF16)


_FWD, _INV = _dft_matrices(CHUNK)
_NT = (((1,), (1,)), ((), ()))


def _interleave(*jobs):
    order = sorted(((i + 0.5) / n, j) for j, (_, n) in enumerate(jobs) for i in range(n))
    for _, j in order:
        next(jobs[j][0])
    for job, _ in jobs:
        for _ in job:
            pass


def _step_schedule(pairs):
    body = "q0 v0 s1 k0 o7 p2"
    drain = "o7 o6 s1 p2 o5 o4 o3 p1 o2 o1 c0"
    order = [(t[0], g - int(t[1:])) for g in range(pairs) for t in body.split()]
    order += [(t[0], pairs - int(t[1:])) for t in drain.split()]
    return [(op, g) for op, g in order if g >= 0]


def _kernel(
    mem0_hbm, shift_hbm, ssmd_hbm, gate_hbm, fwd_hbm, inv_hbm,
    x_hbm, xseg_hbm, k_hbm, v_hbm, ssm_hbm, wq_hbm, wk_hbm, wv_hbm, wo_hbm,
    out_hbm,
    mem0_ref, shift_ref, ssmd_ref, gate_ref, fwd_ref, inv_ref,
    x_s, xtail_s, k_s, v_s, ssm_s, stage_s, wqkv_s, wo_s,
    kpad_s, xf_s, kf_s, zf_s, tail_s,
    h_s, q_s, kb_s, vb_s, p_s, o_s,
    in_sems, w_sems, out_sem,
    *, seq, dm, heads, dh, nmem, seg,
):
    rows = nmem + seg
    nseg = seq // seg
    pairs = heads // 2
    pw = 2 * dh
    nchunk = seq // CHUNK
    nblk = dm // LANES
    w_hbm = (wq_hbm, wk_hbm, wv_hbm)

    def block_copies(j):
        ch = pl.ds(pl.multiple_of(j * LANES, LANES), LANES)
        return [
            pltpu.make_async_copy(src, dst, in_sems.at[3 * j + i])
            for i, (src, dst) in enumerate((
                (ssm_hbm.at[ch, :], ssm_s.at[ch, :]),
                (k_hbm.at[:, ch], k_s.at[:, ch]),
                (v_hbm.at[:, ch], v_s.at[:, ch])))
        ]

    x_copy = pltpu.make_async_copy(x_hbm, x_s, in_sems.at[3 * nblk])
    xtail_copy = pltpu.make_async_copy(
        xseg_hbm.at[:, pl.ds(seg - 8, 8), :], xtail_s, in_sems.at[3 * nblk + 1])

    def w_copy(m, g):
        sl = pl.ds(pl.multiple_of(g * pw, pw), pw)
        if m == 3:
            return pltpu.make_async_copy(
                wo_hbm.at[sl, :], wo_s.at[sl, :], w_sems.at[m * pairs + g])
        return pltpu.make_async_copy(
            w_hbm[m].at[sl, :], stage_s.at[m, g], w_sems.at[m * pairs + g])

    def start_qkv(g):
        for m in range(3):
            w_copy(m, g).start()

    def start_block(j):
        for c in block_copies(j):
            c.start()

    ahead = 2
    small_copies = [
        pltpu.make_async_copy(src, dst, in_sems.at[3 * nblk + 2 + i])
        for i, (src, dst) in enumerate((
            (mem0_hbm, mem0_ref), (shift_hbm, shift_ref), (ssmd_hbm, ssmd_ref),
            (gate_hbm, gate_ref), (fwd_hbm, fwd_ref), (inv_hbm, inv_ref)))
    ]
    for c in small_copies:
        c.start()
    start_block(0)
    start_block(1)
    xtail_copy.start()
    for c in small_copies:
        c.wait()
    kpad_s[0:8, :] = jnp.zeros((8, LANES), F32)
    sub = lax.broadcasted_iota(I32, (8, LANES), 0)
    sign = jnp.where((sub & 1) == 0, 1.0, -1.0).astype(F32)

    def spectra(j, carry):
        for c in block_copies(j):
            c.wait()
        pl.when(j + 2 < nblk)(lambda: start_block(j + 2))
        pl.when(j + ahead >= nblk)(lambda: start_qkv(j + ahead - nblk))

        ch = pl.ds(pl.multiple_of(j * LANES, LANES), LANES)
        fwd = fwd_ref[...]
        kpad_s[8:, :] = k_s[:, ch].astype(F32)
        taps = shift_ref[:, ch].astype(F32)
        prev = None
        for a in range(nchunk):
            t = slice(a * CHUNK, (a + 1) * CHUNK)
            spec = lax.dot_general(
                fwd, ssm_s[ch, t], _NT, preferred_element_type=F32
            ).reshape(CHUNK // 8, 2, 8, LANES)
            if prev is None:
                folded = spec
            else:
                folded = jnp.stack(
                    [spec[:, 0] - sign * prev[:, 1], spec[:, 1] + sign * prev[:, 0]],
                    axis=1)
            kf_s[j, a, 0:2 * CHUNK, :] = folded.reshape(2 * CHUNK, LANES)
            prev = spec
            acc = kpad_s[pl.ds(8 + a * CHUNK, CHUNK), :] * taps[0:1, :]
            for lag in range(1, taps.shape[0]):
                acc = acc + (
                    kpad_s[pl.ds(8 + a * CHUNK - lag, CHUNK), :] * taps[lag:lag + 1, :])
            kv = (acc * v_s[t, ch].astype(F32)).astype(BF16)
            v_s[t, ch] = kv
            xf_s[j, a, 0:2 * CHUNK, :] = jnp.dot(fwd, kv, preferred_element_type=F32)
        return carry

    lax.fori_loop(0, nblk, spectra, 0)
    xtail_copy.wait()

    for s in range(nseg):
        tail_s[8 * s:8 * s + 8, :] = xtail_s[s].astype(F32)

    tail_rows = 128

    def prepare(g, carry):
        for m in range(3):
            w_copy(m, g).wait()
        pl.when(g + ahead < pairs)(lambda: start_qkv(g + ahead))
        w_copy(3, g).start()
        pl.when(g + ahead + 1 == pairs)(x_copy.start)

        last = [None]

        def tail_projection():
            for m in range(2):
                for n in range(pw // LANES):
                    w = stage_s[m, g, n * LANES:(n + 1) * LANES, :]
                    for r in range(0, 8 * nseg, tail_rows):
                        full = lax.dot_general(
                            tail_s[r:r + tail_rows, :], w, _NT, preferred_element_type=F32)
                        for i in range(0, tail_rows, 16):
                            word = (r + i) // 2
                            last[0] = pltpu.bitcast(full[i:i + 16].astype(BF16), F32)
                            kf_s[nblk + 3 * m + n, g, word:word + 8, :] = last[0]
                            yield

        def transpose():
            for m in range(3):
                for n in range(pw // LANES):
                    w = stage_s[m, g, n * LANES:(n + 1) * LANES, :]
                    wqkv_s[g, 0:dm // 2, m * pw + n * LANES:m * pw + (n + 1) * LANES] = (
                        pltpu.bitcast(w.T, I32))
                    wqkv_s[pairs - 1 - g, dm // 2:, 0:LANES] = pltpu.bitcast(last[0], I32)
                    yield

        def chunk_conv():
            re = pl.ds(pl.multiple_of(g * 16, 8), 8)
            im = pl.ds(pl.multiple_of(g * 16 + 8, 8), 8)
            for j in range(nblk):
                xr, xi = [], []
                for c0 in range(0, nchunk, 4):
                    outs = range(c0, c0 + 4)
                    xr += [xf_s[j, c, re, :] for c in outs]
                    xi += [xf_s[j, c, im, :] for c in outs]
                    z = {}
                    for d in range(c0 + 4):
                        kr = kf_s[j, d, re, :]
                        ki = kf_s[j, d, im, :]
                        for c in range(max(c0, d), c0 + 4):
                            tr = xr[c - d] * kr - xi[c - d] * ki
                            ti = xr[c - d] * ki + xi[c - d] * kr
                            z[c] = (z[c][0] + tr, z[c][1] + ti) if d else (tr, ti)
                            yield
                    for c in outs:
                        zf_s[j, c, pl.ds(pl.multiple_of(g * 8, 8), 8), :] = pltpu.bitcast(
                            jnp.concatenate(z[c], axis=0).astype(BF16), I32)

        _interleave(
            (tail_projection(), 2 * (pw // LANES) * nseg // 2),
            (chunk_conv(), nblk * nchunk * (nchunk + 1) // 2),
            (transpose(), 3 * (pw // LANES)),
        )
        return carry

    lax.fori_loop(0, pairs, prepare, 0)

    x_copy.wait()
    for g in range(pairs):
        w_copy(3, g).wait()

    scale = dh ** -0.5
    head = rows - 8
    lane = lax.broadcasted_iota(I32, (rows, LANES), 1)
    first_half = lane < (dh - LANES)
    col = lax.broadcasted_iota(I32, (rows, 2 * rows), 1)
    row = lax.broadcasted_iota(I32, (rows, 2 * rows), 0)
    head0 = col < rows
    allowed = (row < nmem) | (row >= jnp.where(head0, col, col - rows))
    zeros = jnp.zeros((rows, LANES), F32)
    gate_w = gate_ref[...].astype(F32).reshape(1, dm)
    skip = ssmd_ref[...].astype(F32).reshape(1, dm)
    out_s = k_s

    def block_diag(t):
        a, b, c = t[:, :LANES], t[:, LANES:2 * LANES], t[:, 2 * LANES:]
        top = jnp.concatenate([a, jnp.where(first_half, b, 0.0), zeros], axis=1)
        bot = jnp.concatenate([zeros, jnp.where(first_half, 0.0, b), c], axis=1)
        return pltpu.bitcast(jnp.concatenate([top, bot], axis=0).astype(BF16), I32)

    def project_qk(m, g, s):
        two = pl.ds(pl.multiple_of((s // 2) * 8, 8), 8)
        w = pltpu.bitcast(wqkv_s[g, 0:dm // 2, m * pw:(m + 1) * pw], BF16)
        most = jnp.dot(h_s[0:head, :], w, preferred_element_type=F32)
        words = [kf_s[nblk + 3 * m + n, g, two, :] for n in range(pw // LANES)]
        both = pltpu.bitcast(jnp.concatenate(words, axis=1), BF16).astype(F32)
        tail = jnp.where(s % 2 == 0, both[:8], both[8:])
        return jnp.concatenate([most, tail], axis=0)

    def queries(g, s):
        q_s[g] = project_qk(0, g, s)

    def keys(g, s):
        kb_s[g] = block_diag(project_qk(1, g, s))

    def vals(g, s):
        w = pltpu.bitcast(wqkv_s[g, 0:dm // 2, 2 * pw:], BF16)
        vb_s[g] = block_diag(jnp.dot(h_s[...], w, preferred_element_type=F32))

    def scores(g, s):
        sc = lax.dot_general(
            q_s[g], pltpu.bitcast(kb_s[g], BF16), _NT, preferred_element_type=F32)
        sc = jnp.where(allowed, sc * scale, -1000000000.0)
        m0 = jnp.max(jnp.where(head0, sc, -jnp.inf), axis=1, keepdims=True)
        m1 = jnp.max(jnp.where(head0, -jnp.inf, sc), axis=1, keepdims=True)
        e = jnp.exp(sc - jnp.where(head0, m0, m1))
        d0 = jnp.sum(jnp.where(head0, e, 0.0), axis=1, keepdims=True)
        d1 = jnp.sum(jnp.where(head0, 0.0, e), axis=1, keepdims=True)
        p_s[g] = e / jnp.where(head0, d0, d1)

    def weighted(g, s):
        o_s[:, g * pw:(g + 1) * pw] = jnp.dot(
            p_s[g], pltpu.bitcast(vb_s[g], BF16), preferred_element_type=F32)

    def out_proj(g):
        return jnp.dot(
            o_s[:, g * pw:(g + 1) * pw], wo_s[g * pw:(g + 1) * pw, :],
            preferred_element_type=F32)

    def long_conv(s, xs):
        per_chunk = CHUNK // seg
        inv = inv_ref[pl.ds(pl.multiple_of((s % per_chunk) * seg, seg), seg), :]
        spec = jnp.concatenate(
            [zf_s[j, s // per_chunk] for j in range(nblk)], axis=1)
        y = jnp.dot(inv, pltpu.bitcast(spec, BF16), preferred_element_type=F32)
        kv = v_s[pl.ds(pl.multiple_of(s * seg, seg), seg), :].astype(F32)
        return xs * (y + kv * skip)

    h_s[0:nmem, :] = mem0_ref[...].astype(F32)

    def segment(s, carry):
        t = pl.ds(pl.multiple_of(s * seg, seg), seg)
        xs = x_s[t, :].astype(F32)
        h_s[nmem:, :] = xs
        a = b = None
        for op, g in _step_schedule(pairs):
            if op == "o":
                a = out_proj(g) if a is None else a + out_proj(g)
            elif op == "c":
                b = long_conv(s, xs)
            else:
                dict(q=queries, k=keys, v=vals, s=scores, p=weighted)[op](g, s)
        h_s[0:nmem, :] = a[:nmem]
        gate = jax.nn.sigmoid(jnp.sum(xs * gate_w, axis=1, keepdims=True))
        out_s[t, :] = (gate * a[nmem:] + (1.0 - gate) * b).astype(BF16)
        pltpu.make_async_copy(out_s.at[t, :], out_hbm.at[t, :], out_sem).start()
        return carry

    lax.fori_loop(0, nseg, segment, 0, unroll=2)
    pltpu.make_async_copy(out_s, out_hbm, out_sem).wait()


@functools.partial(jax.jit, static_argnames=("A_seg_len",))
def pallas_gated_mix__memory_aug_recurrent_mem_tr__ssm_conv_h3__prompt_kernel(
    A_x: jax.Array,
    A_mem0: jax.Array,
    A_Wq: jax.Array,
    A_Wk: jax.Array,
    A_Wv: jax.Array,
    A_Wo: jax.Array,
    A_seg_len: int,
    B_q: jax.Array,
    B_k: jax.Array,
    B_v: jax.Array,
    B_shift_k: jax.Array,
    B_ssm_k: jax.Array,
    B_ssm_D: jax.Array,
    gate_w: jax.Array,
):
    del B_q
    batch, seq, dm = A_x.shape
    _, heads, dh = A_Wq.shape
    nmem = A_mem0.shape[1]
    seg = int(A_seg_len)
    feat = heads * dh
    rows = nmem + seg
    pairs = heads // 2
    pw = 2 * dh
    nchunk = seq // CHUNK
    nblk = dm // LANES
    nseg = seq // seg
    assert pairs == CHUNK // 8 and nseg % 2 == 0 and CHUNK % seg == 0
    assert batch == 1 and dh == 192 and heads % 8 == 0 and dm % LANES == 0
    assert nmem % 8 == 0 and seg % 16 == 0 and seq % seg == 0 and 2 * rows <= LANES
    assert seq % CHUNK == 0 and B_shift_k.shape[1] <= 8

    def feature_major(w):
        return w.transpose(1, 2, 0).reshape(feat, dm)

    hbm = pl.BlockSpec(memory_space=pltpu.HBM)
    out = pl.pallas_call(
        functools.partial(
            _kernel, seq=seq, dm=dm, heads=heads, dh=dh, nmem=nmem, seg=seg),
        out_shape=jax.ShapeDtypeStruct((seq, dm), BF16),
        in_specs=[hbm] * 15,
        out_specs=hbm,
        scratch_shapes=[
            pltpu.VMEM((nmem, dm), BF16),
            pltpu.VMEM(B_shift_k.shape[::-1], BF16),
            pltpu.VMEM((dm,), BF16),
            pltpu.VMEM((dm,), BF16),
            pltpu.VMEM(_FWD.shape, BF16),
            pltpu.VMEM(_INV.shape, BF16),
            pltpu.VMEM((seq, dm), BF16),
            pltpu.VMEM((nseg, 8, dm), BF16),
            pltpu.VMEM((seq, dm), BF16),
            pltpu.VMEM((seq, dm), BF16),
            pltpu.VMEM((dm, seq), BF16),
            pltpu.VMEM((3, pairs, pw, dm), BF16),
            pltpu.VMEM((pairs, dm // 2 + 8, 3 * pw), I32),
            pltpu.VMEM((feat, dm), BF16),
            pltpu.VMEM((8 + seq, LANES), F32),
            pltpu.VMEM((nblk, nchunk, 2 * CHUNK + 8, LANES), F32),
            pltpu.VMEM((nblk + 6, nchunk, 2 * CHUNK + 24, LANES), F32),
            pltpu.VMEM((nblk, nchunk, CHUNK, LANES), I32),
            pltpu.VMEM((8 * nseg, dm), F32),
            pltpu.VMEM((rows, dm), F32),
            pltpu.VMEM((pairs, rows, pw), F32),
            pltpu.VMEM((pairs, rows, pw), I32),
            pltpu.VMEM((pairs, rows, pw), I32),
            pltpu.VMEM((pairs, rows, 2 * rows), F32),
            pltpu.VMEM((rows, feat), F32),
            pltpu.SemaphoreType.DMA((3 * nblk + 8,)),
            pltpu.SemaphoreType.DMA((4 * pairs,)),
            pltpu.SemaphoreType.DMA,
        ],
        compiler_params=pltpu.CompilerParams(vmem_limit_bytes=112 * 1024 * 1024),
        name="gated_mix_mem_h3",
    )(
        A_mem0.reshape(nmem, dm),
        B_shift_k.T,
        B_ssm_D,
        gate_w,
        _FWD,
        _INV,
        A_x.reshape(seq, dm),
        A_x.reshape(nseg, seg, dm),
        B_k.reshape(seq, dm),
        B_v.reshape(seq, dm),
        B_ssm_k,
        feature_major(A_Wq),
        feature_major(A_Wk),
        feature_major(A_Wv),
        A_Wo.reshape(feat, dm),
    )
    return out.reshape(batch, seq, dm)
```

```python
import functools

import jax
import jax.experimental.pallas as pl
import jax.experimental.pallas.tpu as pltpu
import jax.numpy as jnp
import numpy as np
from jax import lax

F32 = jnp.float32
BF16 = jnp.bfloat16
I32 = jnp.int32
LANES = 128
CHUNK = 128


def _dft_matrices(c):
    theta = np.pi * (np.arange(c)[:, None] + 0.5) * np.arange(c)[None, :] / c
    parts = np.stack([np.cos(theta), -np.sin(theta)])
    fwd = parts.reshape(2, c // 8, 8, c).transpose(1, 0, 2, 3).reshape(2 * c, c)
    return fwd.astype(BF16), (fwd.T / c).astype(BF16)


_FWD, _INV = _dft_matrices(CHUNK)
_NT = (((1,), (1,)), ((), ()))


def _interleave(*jobs):
    order = sorted(((i + 0.5) / n, j) for j, (_, n) in enumerate(jobs) for i in range(n))
    for _, j in order:
        next(jobs[j][0])
    for job, _ in jobs:
        for _ in job:
            pass


def _step_schedule(pairs):
    body = "q0 v0 s1 k0 o7 p2"
    drain = "o7 o6 s1 p2 o5 o4 o3 p1 o2 o1 c0"
    order = [(t[0], g - int(t[1:])) for g in range(pairs) for t in body.split()]
    order += [(t[0], pairs - int(t[1:])) for t in drain.split()]
    return [(op, g) for op, g in order if g >= 0]


def _kernel(
    mem0_hbm, shift_hbm, ssmd_hbm, gate_hbm, fwd_hbm, inv_hbm,
    x_hbm, xseg_hbm, k_hbm, v_hbm, ssm_hbm, wq_hbm, wk_hbm, wv_hbm, wo_hbm,
    out_hbm,
    mem0_ref, shift_ref, ssmd_ref, gate_ref, fwd_ref, inv_ref,
    x_s, xtail_s, k_s, v_s, ssm_s, stage_s, wqkv_s, wo_s,
    kpad_s, xf_s, kf_s, zf_s, tail_s,
    h_s, q_s, kb_s, vb_s, p_s, o_s,
    in_sems, w_sems, out_sem,
    *, seq, dm, heads, dh, nmem, seg,
):
    rows = nmem + seg
    nseg = seq // seg
    pairs = heads // 2
    pw = 2 * dh
    nchunk = seq // CHUNK
    nblk = dm // LANES
    w_hbm = (wq_hbm, wk_hbm, wv_hbm)

    def block_copies(j):
        ch = pl.ds(pl.multiple_of(j * LANES, LANES), LANES)
        return [
            pltpu.make_async_copy(src, dst, in_sems.at[3 * j + i])
            for i, (src, dst) in enumerate((
                (ssm_hbm.at[ch, :], ssm_s.at[ch, :]),
                (k_hbm.at[:, ch], k_s.at[:, ch]),
                (v_hbm.at[:, ch], v_s.at[:, ch])))
        ]

    x_copy = pltpu.make_async_copy(x_hbm, x_s, in_sems.at[3 * nblk])
    xtail_copy = pltpu.make_async_copy(
        xseg_hbm.at[:, pl.ds(seg - 8, 8), :], xtail_s, in_sems.at[3 * nblk + 1])

    def w_copy(m, g):
        sl = pl.ds(pl.multiple_of(g * pw, pw), pw)
        if m == 3:
            return pltpu.make_async_copy(
                wo_hbm.at[sl, :], wo_s.at[sl, :], w_sems.at[m * pairs + g])
        return pltpu.make_async_copy(
            w_hbm[m].at[sl, :], stage_s.at[m, g], w_sems.at[m * pairs + g])

    def start_qkv(g):
        for m in range(3):
            w_copy(m, g).start()

    def start_block(j):
        for c in block_copies(j):
            c.start()

    ahead = 2
    small_copies = [
        pltpu.make_async_copy(src, dst, in_sems.at[3 * nblk + 2 + i])
        for i, (src, dst) in enumerate((
            (mem0_hbm, mem0_ref), (shift_hbm, shift_ref), (ssmd_hbm, ssmd_ref),
            (gate_hbm, gate_ref), (fwd_hbm, fwd_ref), (inv_hbm, inv_ref)))
    ]
    for c in small_copies:
        c.start()
    start_block(0)
    start_block(1)
    xtail_copy.start()
    for c in small_copies:
        c.wait()
    kpad_s[0:8, :] = jnp.zeros((8, LANES), F32)
    sub = lax.broadcasted_iota(I32, (8, LANES), 0)
    sign = jnp.where((sub & 1) == 0, 1.0, -1.0).astype(F32)

    def spectra(j, carry):
        for c in block_copies(j):
            c.wait()
        pl.when(j + 2 < nblk)(lambda: start_block(j + 2))
        pl.when(j + ahead >= nblk)(lambda: start_qkv(j + ahead - nblk))

        ch = pl.ds(pl.multiple_of(j * LANES, LANES), LANES)
        fwd = fwd_ref[...]
        kpad_s[8:, :] = k_s[:, ch].astype(F32)
        taps = shift_ref[:, ch].astype(F32)
        prev = None
        for a in range(nchunk):
            t = slice(a * CHUNK, (a + 1) * CHUNK)
            spec = lax.dot_general(
                fwd, ssm_s[ch, t], _NT, preferred_element_type=F32
            ).reshape(CHUNK // 8, 2, 8, LANES)
            if prev is None:
                folded = spec
            else:
                folded = jnp.stack(
                    [spec[:, 0] - sign * prev[:, 1], spec[:, 1] + sign * prev[:, 0]],
                    axis=1)
            kf_s[j, a] = folded.reshape(2 * CHUNK, LANES)
            prev = spec
            acc = kpad_s[pl.ds(8 + a * CHUNK, CHUNK), :] * taps[0:1, :]
            for lag in range(1, taps.shape[0]):
                acc = acc + (
                    kpad_s[pl.ds(8 + a * CHUNK - lag, CHUNK), :] * taps[lag:lag + 1, :])
            kv = (acc * v_s[t, ch].astype(F32)).astype(BF16)
            v_s[t, ch] = kv
            xf_s[j, a] = jnp.dot(fwd, kv, preferred_element_type=F32)
        return carry

    lax.fori_loop(0, nblk, spectra, 0)
    xtail_copy.wait()

    for s in range(nseg):
        tail_s[8 * s:8 * s + 8, :] = xtail_s[s].astype(F32)

    tail_rows = 256

    def prepare(g, carry):
        for m in range(3):
            w_copy(m, g).wait()
        pl.when(g + ahead < pairs)(lambda: start_qkv(g + ahead))
        w_copy(3, g).start()
        pl.when(g + ahead + 1 == pairs)(x_copy.start)

        last = [None]

        def tail_projection():
            for m in range(2):
                for n in range(pw // LANES):
                    w = stage_s[m, g, n * LANES:(n + 1) * LANES, :]
                    for r in range(0, 8 * nseg, tail_rows):
                        full = lax.dot_general(
                            tail_s[r:r + tail_rows, :], w, _NT, preferred_element_type=F32)
                        for i in range(0, tail_rows, 16):
                            word = (r + i) // 2
                            last[0] = pltpu.bitcast(full[i:i + 16].astype(BF16), F32)
                            kf_s[nblk + 3 * m + n, g, word:word + 8, :] = last[0]
                            yield

        def transpose():
            for m in range(3):
                for n in range(pw // LANES):
                    w = stage_s[m, g, n * LANES:(n + 1) * LANES, :]
                    wqkv_s[g, 0:dm // 2, m * pw + n * LANES:m * pw + (n + 1) * LANES] = (
                        pltpu.bitcast(w.T, I32))
                    wqkv_s[pairs - 1 - g, dm // 2:, 0:LANES] = pltpu.bitcast(last[0], I32)
                    yield

        def chunk_conv():
            re = pl.ds(pl.multiple_of(g * 16, 8), 8)
            im = pl.ds(pl.multiple_of(g * 16 + 8, 8), 8)
            for j in range(nblk):
                xr, xi = [], []
                for c0 in range(0, nchunk, 4):
                    outs = range(c0, c0 + 4)
                    xr += [xf_s[j, c, re, :] for c in outs]
                    xi += [xf_s[j, c, im, :] for c in outs]
                    z = {}
                    for d in range(c0 + 4):
                        kr = kf_s[j, d, re, :]
                        ki = kf_s[j, d, im, :]
                        for c in range(max(c0, d), c0 + 4):
                            tr = xr[c - d] * kr - xi[c - d] * ki
                            ti = xr[c - d] * ki + xi[c - d] * kr
                            z[c] = (z[c][0] + tr, z[c][1] + ti) if d else (tr, ti)
                            yield
                    for c in outs:
                        zf_s[j, c, pl.ds(pl.multiple_of(g * 8, 8), 8), :] = pltpu.bitcast(
                            jnp.concatenate(z[c], axis=0).astype(BF16), I32)

        _interleave(
            (tail_projection(), 2 * (pw // LANES) * nseg // 2),
            (chunk_conv(), nblk * nchunk * (nchunk + 1) // 2),
            (transpose(), 3 * (pw // LANES)),
        )
        return carry

    lax.fori_loop(0, pairs, prepare, 0)

    x_copy.wait()
    for g in range(pairs):
        w_copy(3, g).wait()

    scale = dh ** -0.5
    head = rows - 8
    lane = lax.broadcasted_iota(I32, (rows, LANES), 1)
    first_half = lane < (dh - LANES)
    col = lax.broadcasted_iota(I32, (rows, 2 * rows), 1)
    row = lax.broadcasted_iota(I32, (rows, 2 * rows), 0)
    head0 = col < rows
    allowed = (row < nmem) | (row >= jnp.where(head0, col, col - rows))
    zeros = jnp.zeros((rows, LANES), F32)
    gate_w = gate_ref[...].astype(F32).reshape(1, dm)
    skip = ssmd_ref[...].astype(F32).reshape(1, dm)
    out_s = k_s

    def block_diag(t):
        a, b, c = t[:, :LANES], t[:, LANES:2 * LANES], t[:, 2 * LANES:]
        top = jnp.concatenate([a, jnp.where(first_half, b, 0.0), zeros], axis=1)
        bot = jnp.concatenate([zeros, jnp.where(first_half, 0.0, b), c], axis=1)
        return pltpu.bitcast(jnp.concatenate([top, bot], axis=0).astype(BF16), I32)

    def project_qk(m, g, s):
        two = pl.ds(pl.multiple_of((s // 2) * 8, 8), 8)
        w = pltpu.bitcast(wqkv_s[g, 0:dm // 2, m * pw:(m + 1) * pw], BF16)
        most = jnp.dot(h_s[0:head, :], w, preferred_element_type=F32)
        words = [kf_s[nblk + 3 * m + n, g, two, :] for n in range(pw // LANES)]
        both = pltpu.bitcast(jnp.concatenate(words, axis=1), BF16).astype(F32)
        tail = jnp.where(s % 2 == 0, both[:8], both[8:])
        return jnp.concatenate([most, tail], axis=0)

    def queries(g, s):
        q_s[g] = project_qk(0, g, s)

    def keys(g, s):
        kb_s[g] = block_diag(project_qk(1, g, s))

    def vals(g, s):
        w = pltpu.bitcast(wqkv_s[g, 0:dm // 2, 2 * pw:], BF16)
        vb_s[g] = block_diag(jnp.dot(h_s[...], w, preferred_element_type=F32))

    def scores(g, s):
        sc = lax.dot_general(
            q_s[g], pltpu.bitcast(kb_s[g], BF16), _NT, preferred_element_type=F32)
        sc = jnp.where(allowed, sc * scale, -1000000000.0)
        m0 = jnp.max(jnp.where(head0, sc, -jnp.inf), axis=1, keepdims=True)
        m1 = jnp.max(jnp.where(head0, -jnp.inf, sc), axis=1, keepdims=True)
        e = jnp.exp(sc - jnp.where(head0, m0, m1))
        d0 = jnp.sum(jnp.where(head0, e, 0.0), axis=1, keepdims=True)
        d1 = jnp.sum(jnp.where(head0, 0.0, e), axis=1, keepdims=True)
        p_s[g] = e / jnp.where(head0, d0, d1)

    def weighted(g, s):
        o_s[:, g * pw:(g + 1) * pw] = jnp.dot(
            p_s[g], pltpu.bitcast(vb_s[g], BF16), preferred_element_type=F32)

    def out_proj(g):
        return jnp.dot(
            o_s[:, g * pw:(g + 1) * pw], wo_s[g * pw:(g + 1) * pw, :],
            preferred_element_type=F32)

    def long_conv(s, xs):
        per_chunk = CHUNK // seg
        inv = inv_ref[pl.ds(pl.multiple_of((s % per_chunk) * seg, seg), seg), :]
        spec = jnp.concatenate(
            [zf_s[j, s // per_chunk] for j in range(nblk)], axis=1)
        y = jnp.dot(inv, pltpu.bitcast(spec, BF16), preferred_element_type=F32)
        kv = v_s[pl.ds(pl.multiple_of(s * seg, seg), seg), :].astype(F32)
        return xs * (y + kv * skip)

    h_s[0:nmem, :] = mem0_ref[...].astype(F32)

    def segment(s, carry):
        t = pl.ds(pl.multiple_of(s * seg, seg), seg)
        xs = x_s[t, :].astype(F32)
        h_s[nmem:, :] = xs
        a = b = None
        for op, g in _step_schedule(pairs):
            if op == "o":
                a = out_proj(g) if a is None else a + out_proj(g)
            elif op == "c":
                b = long_conv(s, xs)
            else:
                dict(q=queries, k=keys, v=vals, s=scores, p=weighted)[op](g, s)
        h_s[0:nmem, :] = a[:nmem]
        gate = jax.nn.sigmoid(jnp.sum(xs * gate_w, axis=1, keepdims=True))
        out_s[t, :] = (gate * a[nmem:] + (1.0 - gate) * b).astype(BF16)
        pltpu.make_async_copy(out_s.at[t, :], out_hbm.at[t, :], out_sem).start()
        return carry

    lax.fori_loop(0, nseg, segment, 0, unroll=2)
    pltpu.make_async_copy(out_s, out_hbm, out_sem).wait()


@functools.partial(jax.jit, static_argnames=("A_seg_len",))
def pallas_gated_mix__memory_aug_recurrent_mem_tr__ssm_conv_h3__prompt_kernel(
    A_x: jax.Array,
    A_mem0: jax.Array,
    A_Wq: jax.Array,
    A_Wk: jax.Array,
    A_Wv: jax.Array,
    A_Wo: jax.Array,
    A_seg_len: int,
    B_q: jax.Array,
    B_k: jax.Array,
    B_v: jax.Array,
    B_shift_k: jax.Array,
    B_ssm_k: jax.Array,
    B_ssm_D: jax.Array,
    gate_w: jax.Array,
):
    del B_q
    batch, seq, dm = A_x.shape
    _, heads, dh = A_Wq.shape
    nmem = A_mem0.shape[1]
    seg = int(A_seg_len)
    feat = heads * dh
    rows = nmem + seg
    pairs = heads // 2
    pw = 2 * dh
    nchunk = seq // CHUNK
    nblk = dm // LANES
    nseg = seq // seg
    assert pairs == CHUNK // 8 and nseg % 2 == 0 and CHUNK % seg == 0
    assert batch == 1 and dh == 192 and heads % 8 == 0 and dm % LANES == 0
    assert nmem % 8 == 0 and seg % 16 == 0 and seq % seg == 0 and 2 * rows <= LANES
    assert seq % CHUNK == 0 and B_shift_k.shape[1] <= 8

    def feature_major(w):
        return w.transpose(1, 2, 0).reshape(feat, dm)

    hbm = pl.BlockSpec(memory_space=pltpu.HBM)
    out = pl.pallas_call(
        functools.partial(
            _kernel, seq=seq, dm=dm, heads=heads, dh=dh, nmem=nmem, seg=seg),
        out_shape=jax.ShapeDtypeStruct((seq, dm), BF16),
        in_specs=[hbm] * 15,
        out_specs=hbm,
        scratch_shapes=[
            pltpu.VMEM((nmem, dm), BF16),
            pltpu.VMEM(B_shift_k.shape[::-1], BF16),
            pltpu.VMEM((dm,), BF16),
            pltpu.VMEM((dm,), BF16),
            pltpu.VMEM(_FWD.shape, BF16),
            pltpu.VMEM(_INV.shape, BF16),
            pltpu.VMEM((seq, dm), BF16),
            pltpu.VMEM((nseg, 8, dm), BF16),
            pltpu.VMEM((seq, dm), BF16),
            pltpu.VMEM((seq, dm), BF16),
            pltpu.VMEM((dm, seq), BF16),
            pltpu.VMEM((3, pairs, pw, dm), BF16),
            pltpu.VMEM((pairs, dm // 2 + 8, 3 * pw), I32),
            pltpu.VMEM((feat, dm), BF16),
            pltpu.VMEM((8 + seq, LANES), F32),
            pltpu.VMEM((nblk, nchunk, 2 * CHUNK, LANES), F32),
            pltpu.VMEM((nblk + 6, nchunk, 2 * CHUNK, LANES), F32),
            pltpu.VMEM((nblk, nchunk, CHUNK, LANES), I32),
            pltpu.VMEM((8 * nseg, dm), F32),
            pltpu.VMEM((rows, dm), F32),
            pltpu.VMEM((pairs, rows, pw), F32),
            pltpu.VMEM((pairs, rows, pw), I32),
            pltpu.VMEM((pairs, rows, pw), I32),
            pltpu.VMEM((pairs, rows, 2 * rows), F32),
            pltpu.VMEM((rows, feat), F32),
            pltpu.SemaphoreType.DMA((3 * nblk + 8,)),
            pltpu.SemaphoreType.DMA((4 * pairs,)),
            pltpu.SemaphoreType.DMA,
        ],
        compiler_params=pltpu.CompilerParams(vmem_limit_bytes=112 * 1024 * 1024),
        name="gated_mix_mem_h3",
    )(
        A_mem0.reshape(nmem, dm),
        B_shift_k.T,
        B_ssm_D,
        gate_w,
        _FWD,
        _INV,
        A_x.reshape(seq, dm),
        A_x.reshape(nseg, seg, dm),
        B_k.reshape(seq, dm),
        B_v.reshape(seq, dm),
        B_ssm_k,
        feature_major(A_Wq),
        feature_major(A_Wk),
        feature_major(A_Wv),
        A_Wo.reshape(feat, dm),
    )
    return out.reshape(batch, seq, dm)
```

```python
import functools

import jax
import jax.experimental.pallas as pl
import jax.experimental.pallas.tpu as pltpu
import jax.numpy as jnp
import numpy as np
from jax import lax

F32 = jnp.float32
BF16 = jnp.bfloat16
I32 = jnp.int32
LANES = 128
CHUNK = 128


def _dft_matrices(c):
    theta = np.pi * (np.arange(c)[:, None] + 0.5) * np.arange(c)[None, :] / c
    parts = np.stack([np.cos(theta), -np.sin(theta)])
    fwd = parts.reshape(2, c // 8, 8, c).transpose(1, 0, 2, 3).reshape(2 * c, c)
    return fwd.astype(BF16), (fwd.T / c).astype(BF16)


_FWD, _INV = _dft_matrices(CHUNK)
_NT = (((1,), (1,)), ((), ()))


def _interleave(*jobs):
    order = sorted(((i + 0.5) / n, j) for j, (_, n) in enumerate(jobs) for i in range(n))
    for _, j in order:
        next(jobs[j][0])
    for job, _ in jobs:
        for _ in job:
            pass


def _step_schedule(pairs):
    body = "q0 v0 s1 k0 o7 p2"
    drain = "o7 o6 s1 p2 o5 o4 o3 p1 o2 o1 c0"
    order = [(t[0], g - int(t[1:])) for g in range(pairs) for t in body.split()]
    order += [(t[0], pairs - int(t[1:])) for t in drain.split()]
    return [(op, g) for op, g in order if g >= 0]


def _kernel(
    mem0_hbm, shift_hbm, ssmd_hbm, gate_hbm, fwd_hbm, inv_hbm,
    x_hbm, xseg_hbm, k_hbm, v_hbm, ssm_hbm, wq_hbm, wk_hbm, wv_hbm, wo_hbm,
    out_hbm,
    mem0_ref, shift_ref, ssmd_ref, gate_ref, fwd_ref, inv_ref,
    x_s, xtail_s, k_s, v_s, ssm_s, stage_s, wqkv_s, wo_s,
    kpad_s, xf_s, kf_s, zf_s, tail_s,
    h_s, q_s, kb_s, vb_s, p_s, o_s,
    in_sems, w_sems, out_sem,
    *, seq, dm, heads, dh, nmem, seg,
):
    rows = nmem + seg
    nseg = seq // seg
    pairs = heads // 2
    pw = 2 * dh
    nchunk = seq // CHUNK
    nblk = dm // LANES
    w_hbm = (wq_hbm, wk_hbm, wv_hbm)

    def block_copies(j):
        ch = pl.ds(pl.multiple_of(j * LANES, LANES), LANES)
        return [
            pltpu.make_async_copy(src, dst, in_sems.at[3 * j + i])
            for i, (src, dst) in enumerate((
                (ssm_hbm.at[ch, :], ssm_s.at[ch, :]),
                (k_hbm.at[:, ch], k_s.at[:, ch]),
                (v_hbm.at[:, ch], v_s.at[:, ch])))
        ]

    x_copy = pltpu.make_async_copy(x_hbm, x_s, in_sems.at[3 * nblk])
    xtail_copy = pltpu.make_async_copy(
        xseg_hbm.at[:, pl.ds(seg - 8, 8), :], xtail_s, in_sems.at[3 * nblk + 1])

    def w_copy(m, g):
        sl = pl.ds(pl.multiple_of(g * pw, pw), pw)
        if m == 3:
            return pltpu.make_async_copy(
                wo_hbm.at[sl, :], wo_s.at[sl, :], w_sems.at[m * pairs + g])
        return pltpu.make_async_copy(
            w_hbm[m].at[sl, :], stage_s.at[m, g], w_sems.at[m * pairs + g])

    def start_qkv(g):
        for m in range(3):
            w_copy(m, g).start()

    def start_block(j):
        for c in block_copies(j):
            c.start()

    ahead = 2
    small_copies = [
        pltpu.make_async_copy(src, dst, in_sems.at[3 * nblk + 2 + i])
        for i, (src, dst) in enumerate((
            (mem0_hbm, mem0_ref), (shift_hbm, shift_ref), (ssmd_hbm, ssmd_ref),
            (gate_hbm, gate_ref), (fwd_hbm, fwd_ref), (inv_hbm, inv_ref)))
    ]
    for c in small_copies:
        c.start()
    start_block(0)
    start_block(1)
    xtail_copy.start()
    for c in small_copies:
        c.wait()
    kpad_s[0:8, :] = jnp.zeros((8, LANES), F32)
    sub = lax.broadcasted_iota(I32, (8, LANES), 0)
    sign = jnp.where((sub & 1) == 0, 1.0, -1.0).astype(F32)

    def spectra(j, carry):
        for c in block_copies(j):
            c.wait()
        pl.when(j + 2 < nblk)(lambda: start_block(j + 2))
        pl.when(j + ahead >= nblk)(lambda: start_qkv(j + ahead - nblk))

        ch = pl.ds(pl.multiple_of(j * LANES, LANES), LANES)
        fwd = fwd_ref[...]
        kpad_s[8:, :] = k_s[:, ch].astype(F32)
        taps = shift_ref[:, ch].astype(F32)
        prev = None
        for a in range(nchunk):
            t = slice(a * CHUNK, (a + 1) * CHUNK)
            spec = lax.dot_general(
                fwd, ssm_s[ch, t], _NT, preferred_element_type=F32
            ).reshape(CHUNK // 8, 2, 8, LANES)
            if prev is None:
                folded = spec
            else:
                folded = jnp.stack(
                    [spec[:, 0] - sign * prev[:, 1], spec[:, 1] + sign * prev[:, 0]],
                    axis=1)
            kf_s[j, a] = folded.reshape(2 * CHUNK, LANES)
            prev = spec
            acc = kpad_s[pl.ds(8 + a * CHUNK, CHUNK), :] * taps[0:1, :]
            for lag in range(1, taps.shape[0]):
                acc = acc + (
                    kpad_s[pl.ds(8 + a * CHUNK - lag, CHUNK), :] * taps[lag:lag + 1, :])
            kv = (acc * v_s[t, ch].astype(F32)).astype(BF16)
            v_s[t, ch] = kv
            xf_s[j, a] = jnp.dot(fwd, kv, preferred_element_type=F32)
        return carry

    lax.fori_loop(0, nblk, spectra, 0)
    xtail_copy.wait()

    for s in range(nseg):
        tail_s[8 * s:8 * s + 8, :] = xtail_s[s].astype(F32)

    tail_rows = 256

    def prepare(g, carry):
        for m in range(3):
            w_copy(m, g).wait()
        pl.when(g + ahead < pairs)(lambda: start_qkv(g + ahead))
        w_copy(3, g).start()
        pl.when(g + ahead + 1 == pairs)(x_copy.start)

        last = [None]

        def tail_projection():
            for m in range(2):
                for n in range(pw // LANES):
                    w = stage_s[m, g, n * LANES:(n + 1) * LANES, :]
                    for r in range(0, 8 * nseg, tail_rows):
                        full = lax.dot_general(
                            tail_s[r:r + tail_rows, :], w, _NT, preferred_element_type=F32)
                        for i in range(0, tail_rows, 16):
                            word = (r + i) // 2
                            last[0] = pltpu.bitcast(full[i:i + 16].astype(BF16), F32)
                            kf_s[nblk + 3 * m + n, g, word:word + 8, :] = last[0]
                            yield

        def transpose():
            for m in range(3):
                for n in range(pw // LANES):
                    w = stage_s[m, g, n * LANES:(n + 1) * LANES, :]
                    wqkv_s[g, 0:dm // 2, m * pw + n * LANES:m * pw + (n + 1) * LANES] = (
                        pltpu.bitcast(w.T, I32))
                    wqkv_s[pairs - 1 - g, dm // 2:, 0:LANES] = pltpu.bitcast(last[0], I32)
                    yield

        def chunk_conv():
            re = pl.ds(pl.multiple_of(g * 16, 8), 8)
            im = pl.ds(pl.multiple_of(g * 16 + 8, 8), 8)
            for j in range(nblk):
                xr, xi = [], []
                for c0 in range(0, nchunk, 4):
                    outs = range(c0, c0 + 4)
                    xr += [xf_s[j, c, re, :] for c in outs]
                    xi += [xf_s[j, c, im, :] for c in outs]
                    z = {}
                    for d in range(c0 + 4):
                        kr = kf_s[j, d, re, :]
                        ki = kf_s[j, d, im, :]
                        for c in range(max(c0, d), c0 + 4):
                            tr = xr[c - d] * kr - xi[c - d] * ki
                            ti = xr[c - d] * ki + xi[c - d] * kr
                            z[c] = (z[c][0] + tr, z[c][1] + ti) if d else (tr, ti)
                            yield
                    for c in outs:
                        zf_s[j, c, pl.ds(pl.multiple_of(g * 8, 8), 8), :] = pltpu.bitcast(
                            jnp.concatenate(z[c], axis=0).astype(BF16), I32)

        _interleave(
            (tail_projection(), 2 * (pw // LANES) * 8 * nseg // 16),
            (chunk_conv(), nblk * nchunk * (nchunk + 1) // 2),
            (transpose(), 3 * (pw // LANES)),
        )
        return carry

    lax.fori_loop(0, pairs, prepare, 0)

    x_copy.wait()
    for g in range(pairs):
        w_copy(3, g).wait()

    scale = dh ** -0.5
    head = rows - 8
    lane = lax.broadcasted_iota(I32, (rows, LANES), 1)
    first_half = lane < (dh - LANES)
    col = lax.broadcasted_iota(I32, (rows, 2 * rows), 1)
    row = lax.broadcasted_iota(I32, (rows, 2 * rows), 0)
    head0 = col < rows
    allowed = (row < nmem) | (row >= jnp.where(head0, col, col - rows))
    zeros = jnp.zeros((rows, LANES), F32)
    gate_w = gate_ref[...].astype(F32).reshape(1, dm)
    skip = ssmd_ref[...].astype(F32).reshape(1, dm)
    out_s = k_s

    def block_diag(t):
        a, b, c = t[:, :LANES], t[:, LANES:2 * LANES], t[:, 2 * LANES:]
        top = jnp.concatenate([a, jnp.where(first_half, b, 0.0), zeros], axis=1)
        bot = jnp.concatenate([zeros, jnp.where(first_half, 0.0, b), c], axis=1)
        return pltpu.bitcast(jnp.concatenate([top, bot], axis=0).astype(BF16), I32)

    def project_qk(m, g, s):
        two = pl.ds(pl.multiple_of((s // 2) * 8, 8), 8)
        w = pltpu.bitcast(wqkv_s[g, 0:dm // 2, m * pw:(m + 1) * pw], BF16)
        most = jnp.dot(h_s[0:head, :], w, preferred_element_type=F32)
        words = [kf_s[nblk + 3 * m + n, g, two, :] for n in range(pw // LANES)]
        both = pltpu.bitcast(jnp.concatenate(words, axis=1), BF16).astype(F32)
        tail = jnp.where(s % 2 == 0, both[:8], both[8:])
        return jnp.concatenate([most, tail], axis=0)

    def queries(g, s):
        q_s[g] = project_qk(0, g, s)

    def keys(g, s):
        kb_s[g] = block_diag(project_qk(1, g, s))

    def vals(g, s):
        w = pltpu.bitcast(wqkv_s[g, 0:dm // 2, 2 * pw:], BF16)
        vb_s[g] = block_diag(jnp.dot(h_s[...], w, preferred_element_type=F32))

    def scores(g, s):
        sc = lax.dot_general(
            q_s[g], pltpu.bitcast(kb_s[g], BF16), _NT, preferred_element_type=F32)
        sc = jnp.where(allowed, sc * scale, -1000000000.0)
        m0 = jnp.max(jnp.where(head0, sc, -jnp.inf), axis=1, keepdims=True)
        m1 = jnp.max(jnp.where(head0, -jnp.inf, sc), axis=1, keepdims=True)
        e = jnp.exp(sc - jnp.where(head0, m0, m1))
        d0 = jnp.sum(jnp.where(head0, e, 0.0), axis=1, keepdims=True)
        d1 = jnp.sum(jnp.where(head0, 0.0, e), axis=1, keepdims=True)
        p_s[g] = e / jnp.where(head0, d0, d1)

    def weighted(g, s):
        o_s[:, g * pw:(g + 1) * pw] = jnp.dot(
            p_s[g], pltpu.bitcast(vb_s[g], BF16), preferred_element_type=F32)

    def out_proj(g):
        return jnp.dot(
            o_s[:, g * pw:(g + 1) * pw], wo_s[g * pw:(g + 1) * pw, :],
            preferred_element_type=F32)

    def long_conv(s, xs):
        per_chunk = CHUNK // seg
        inv = inv_ref[pl.ds(pl.multiple_of((s % per_chunk) * seg, seg), seg), :]
        spec = jnp.concatenate(
            [zf_s[j, s // per_chunk] for j in range(nblk)], axis=1)
        y = jnp.dot(inv, pltpu.bitcast(spec, BF16), preferred_element_type=F32)
        kv = v_s[pl.ds(pl.multiple_of(s * seg, seg), seg), :].astype(F32)
        return xs * (y + kv * skip)

    h_s[0:nmem, :] = mem0_ref[...].astype(F32)

    def segment(s, carry):
        t = pl.ds(pl.multiple_of(s * seg, seg), seg)
        xs = x_s[t, :].astype(F32)
        h_s[nmem:, :] = xs
        a = b = None
        for op, g in _step_schedule(pairs):
            if op == "o":
                a = out_proj(g) if a is None else a + out_proj(g)
            elif op == "c":
                b = long_conv(s, xs)
            else:
                dict(q=queries, k=keys, v=vals, s=scores, p=weighted)[op](g, s)
        h_s[0:nmem, :] = a[:nmem]
        gate = jax.nn.sigmoid(jnp.sum(xs * gate_w, axis=1, keepdims=True))
        out_s[t, :] = (gate * a[nmem:] + (1.0 - gate) * b).astype(BF16)
        pltpu.make_async_copy(out_s.at[t, :], out_hbm.at[t, :], out_sem).start()
        return carry

    lax.fori_loop(0, nseg, segment, 0, unroll=2)
    pltpu.make_async_copy(out_s, out_hbm, out_sem).wait()


@functools.partial(jax.jit, static_argnames=("A_seg_len",))
def pallas_gated_mix__memory_aug_recurrent_mem_tr__ssm_conv_h3__prompt_kernel(
    A_x: jax.Array,
    A_mem0: jax.Array,
    A_Wq: jax.Array,
    A_Wk: jax.Array,
    A_Wv: jax.Array,
    A_Wo: jax.Array,
    A_seg_len: int,
    B_q: jax.Array,
    B_k: jax.Array,
    B_v: jax.Array,
    B_shift_k: jax.Array,
    B_ssm_k: jax.Array,
    B_ssm_D: jax.Array,
    gate_w: jax.Array,
):
    del B_q
    batch, seq, dm = A_x.shape
    _, heads, dh = A_Wq.shape
    nmem = A_mem0.shape[1]
    seg = int(A_seg_len)
    feat = heads * dh
    rows = nmem + seg
    pairs = heads // 2
    pw = 2 * dh
    nchunk = seq // CHUNK
    nblk = dm // LANES
    nseg = seq // seg
    assert batch == 1 and dh == 192 and dm % LANES == 0 and 2 * rows <= LANES
    assert nmem % 8 == 0 and seg % 16 == 0 and CHUNK % seg == 0 and seq % CHUNK == 0
    assert pairs == nchunk == CHUNK // 8 and 4 * nseg == 2 * CHUNK
    assert B_shift_k.shape[1] <= 8

    def feature_major(w):
        return w.transpose(1, 2, 0).reshape(feat, dm)

    hbm = pl.BlockSpec(memory_space=pltpu.HBM)
    out = pl.pallas_call(
        functools.partial(
            _kernel, seq=seq, dm=dm, heads=heads, dh=dh, nmem=nmem, seg=seg),
        out_shape=jax.ShapeDtypeStruct((seq, dm), BF16),
        in_specs=[hbm] * 15,
        out_specs=hbm,
        scratch_shapes=[
            pltpu.VMEM((nmem, dm), BF16),
            pltpu.VMEM(B_shift_k.shape[::-1], BF16),
            pltpu.VMEM((dm,), BF16),
            pltpu.VMEM((dm,), BF16),
            pltpu.VMEM(_FWD.shape, BF16),
            pltpu.VMEM(_INV.shape, BF16),
            pltpu.VMEM((seq, dm), BF16),
            pltpu.VMEM((nseg, 8, dm), BF16),
            pltpu.VMEM((seq, dm), BF16),
            pltpu.VMEM((seq, dm), BF16),
            pltpu.VMEM((dm, seq), BF16),
            pltpu.VMEM((3, pairs, pw, dm), BF16),
            pltpu.VMEM((pairs, dm // 2 + 8, 3 * pw), I32),
            pltpu.VMEM((feat, dm), BF16),
            pltpu.VMEM((8 + seq, LANES), F32),
            pltpu.VMEM((nblk, nchunk, 2 * CHUNK, LANES), F32),
            pltpu.VMEM((nblk + 6, nchunk, 2 * CHUNK, LANES), F32),
            pltpu.VMEM((nblk, nchunk, CHUNK, LANES), I32),
            pltpu.VMEM((8 * nseg, dm), F32),
            pltpu.VMEM((rows, dm), F32),
            pltpu.VMEM((pairs, rows, pw), F32),
            pltpu.VMEM((pairs, rows, pw), I32),
            pltpu.VMEM((pairs, rows, pw), I32),
            pltpu.VMEM((pairs, rows, 2 * rows), F32),
            pltpu.VMEM((rows, feat), F32),
            pltpu.SemaphoreType.DMA((3 * nblk + 8,)),
            pltpu.SemaphoreType.DMA((4 * pairs,)),
            pltpu.SemaphoreType.DMA,
        ],
        compiler_params=pltpu.CompilerParams(vmem_limit_bytes=112 * 1024 * 1024),
        name="gated_mix_mem_h3",
    )(
        A_mem0.reshape(nmem, dm),
        B_shift_k.T,
        B_ssm_D,
        gate_w,
        _FWD,
        _INV,
        A_x.reshape(seq, dm),
        A_x.reshape(nseg, seg, dm),
        B_k.reshape(seq, dm),
        B_v.reshape(seq, dm),
        B_ssm_k,
        feature_major(A_Wq),
        feature_major(A_Wk),
        feature_major(A_Wv),
        A_Wo.reshape(feat, dm),
    )
    return out.reshape(batch, seq, dm)
```
